```python
import jax
import jax.numpy as jnp

def _softmax(x, axis=-1):
    return jax.nn.softmax(x, axis=axis)
def _gelu(x):
    return jax.nn.gelu(x, approximate=True)
def _silu(x):
    return jax.nn.silu(x)
def _sigmoid(x):
    return jax.nn.sigmoid(x)
def _layernorm(x, axis=-1, eps=1e-5):
    m = jnp.mean(x, axis=axis, keepdims=True)
    v = jnp.var(x, axis=axis, keepdims=True)
    return (x - m) / jnp.sqrt(v + eps)
def _scatter_add(tgt, idx, src, axis=0):
    return tgt.at[idx].add(src)
def _segment_sum(src, seg, n):
    return jax.ops.segment_sum(src, seg, n)
class _Rng:
    def __init__(self, key):
        self._k = key
    def _next(self):
        self._k, sub = jax.random.split(self._k)
        return sub
    def normal(self, shape):
        return jax.random.normal(self._next(), shape, dtype=jnp.bfloat16)
    def randint(self, lo, hi, shape):
        return jax.random.randint(self._next(), shape, lo, hi, dtype=jnp.int32)
    def uniform(self, shape, lo=0.0, hi=1.0):
        return jax.random.uniform(self._next(), shape, jnp.bfloat16, lo, hi)
    def permutation(self, n):
        return jax.random.permutation(self._next(), n)


kernel_name = 'parallel_sum__linear_attn_block__moe_arch_mod__prompt'

def setup_inputs():
    _rng = _Rng(jax.random.key(int.from_bytes(__import__("os").urandom(4), "little")))
    _w = (lambda a: (lambda t: t.astype(jnp.bfloat16) if jnp.issubdtype(t.dtype, jnp.floating) else t)(jnp.asarray(a)))
    def _A_setup():
        B, S, D = 1, 2048, 1024
        return {
            "x": _w((lambda *s: _rng.normal(s) * 0.05)(B, S, D)),
            "wqkv": _w((lambda *s: _rng.normal(s) * 0.05)(D, 3 * D)),
            "wo": _w((lambda *s: _rng.normal(s) * 0.05)(D, D)),
        }
    _A_in = _A_setup()

    def _B_setup():
        B, S, D, F, C = 1, 2048, 1024, 3584, 1
        return {
            "x": _w((lambda *s: _rng.normal(s) * 0.05)(B, S, D)),
            "w_r": _w((lambda *s: _rng.normal(s) * 0.05)(D)),
            "w_gate": _w((lambda *s: _rng.normal(s) * 0.05)(D, F)),
            "w_up": _w((lambda *s: _rng.normal(s) * 0.05)(D, F)),
            "w_down": _w((lambda *s: _rng.normal(s) * 0.05)(F, D)),
        }
    _B_in = _B_setup()

    return {
        "A_x": _A_in["x"],
        "A_wqkv": _A_in["wqkv"],
        "A_wo": _A_in["wo"],
        "B_x": _B_in["x"],
        "B_w_r": _B_in["w_r"],
        "B_w_gate": _B_in["w_gate"],
        "B_w_up": _B_in["w_up"],
        "B_w_down": _B_in["w_down"],
    }

def reference(A_x, A_wqkv, A_wo, B_x, B_w_r, B_w_gate, B_w_up, B_w_down):
    def _A_ref(x, wqkv, wo):
        B, S, D = x.shape
        H = 32; Dh = D // H
        qkv = (lambda x, *d: x.transpose(*d))((x @ wqkv).reshape(B, S, 3, H, Dh), 2, 0, 3, 1, 4)
        q, k, v = qkv[0], qkv[1], qkv[2]
        phi = lambda t: jnp.where(t > 0, t + 1, jnp.exp(t)) + 1e-6
        pq, pk = phi(q), phi(k)
        kv = jnp.einsum("bhsd,bhse->bhde", pk, v)
        z = jnp.einsum("bhsd->bhd", pk)
        num = jnp.einsum("bhqd,bhde->bhqe", pq, kv)
        den = jnp.einsum("bhqd,bhd->bhq", pq, z)[..., None] + 1e-6
        o = num / den
        return (lambda x, *d: x.transpose(*d))(o, 0, 2, 1, 3).reshape(B, S, D) @ wo

    def _B_ref(x, w_r, w_gate, w_up, w_down):
        B, S, D = x.shape
        C = 1
        r = x @ w_r
        idx = jnp.argsort(-r, axis=-1)[:, :C]
        idx_e = jnp.repeat(idx.reshape(B, C, 1), D, axis=2)
        x_sel = jnp.take_along_axis(x, idx_e, axis=1)
        g = _silu(x_sel @ w_gate)
        u = x_sel @ w_up
        y = (g * u) @ w_down
        r_sel = _sigmoid(jnp.take_along_axis(r, idx, axis=1))
        y = y * r_sel.reshape(B, C, 1)
        b_off = (jnp.arange(B) * S).reshape(B, 1)
        flat_idx = (idx + b_off).reshape(B * C)
        zero = (x * 0.0).reshape(B * S, D)
        upd = _scatter_add(zero, flat_idx, y.reshape(B * C, D), axis=0)
        return x + upd.reshape(B, S, D)

    x = A_x
    xn = _layernorm(x, axis=-1)
    return x + _A_ref(xn, A_wqkv, A_wo) + _B_ref(xn, B_w_r, B_w_gate, B_w_up, B_w_down)
```

```python
import contextlib
import numpy as np
import jax
import jax.numpy as jnp
from jax import lax
from jax.experimental import pallas as pl
from jax.experimental.pallas import tpu as pltpu

S, D, H, DH, F = 2048, 1024, 32, 32, 3584
G = D // 128
BF, F32, U32 = jnp.bfloat16, jnp.float32, jnp.uint32
NN = (((1,), (0,)), ((), ()))
NT = (((1,), (1,)), ((), ()))
TN = (((0,), (0,)), ((), ()))


def _dot(a, b, dn=NN):
    return lax.dot_general(a, b, dn, preferred_element_type=F32)


def _rnd(x):
    return x.astype(BF).astype(F32)


def _phi(t):
    return jnp.where(t > 0, t + 1.0, jnp.exp(t)) + 1e-6


def make_kernel(cfg):
    TS = cfg.get("TS", 512)
    NTILE = S // TS
    LNP = cfg.get("LNP", 128)
    NPT = TS // LNP
    FC = cfg.get("FC", 512)
    NFC = F // FC
    ON = cfg.get("ON", 256)
    NOC = D // ON
    scopes = cfg.get("scopes", False)
    ffn_mode = cfg.get("ffn", "mid")
    packed = cfg.get("packed", True)
    bars = cfg.get("bars", (1, 3, 7, 15))

    def scope(name):
        return jax.named_scope(name) if scopes else contextlib.nullcontext()

    class PB:
        def __init__(self, ref):
            self.ref = ref
        def ld(self, r0, nr, c0=0, nc=None):
            nc = self.ref.shape[1] - c0 if nc is None else nc
            if packed:
                if isinstance(r0, int):
                    v = self.ref[pl.ds(r0 // 2, nr // 2), pl.ds(c0, nc)]
                else:
                    v = self.ref[pl.ds(pl.multiple_of(r0 // 2, 8), nr // 2), pl.ds(c0, nc)]
                return pltpu.bitcast(v, BF)
            return self.ref[pl.ds(r0, nr), pl.ds(c0, nc)]
        def st(self, r0, c0, val):
            nr, nc = val.shape
            if packed:
                self.ref[pl.ds(r0 // 2, nr // 2), pl.ds(c0, nc)] = pltpu.bitcast(val, U32)
            else:
                self.ref[pl.ds(r0, nr), pl.ds(c0, nc)] = val

    def kernel(x_hbm, wqkv_hbm, wo_hbm, wr_hbm, wg_hbm, wu_hbm, wd_hbm, out_hbm,
               x_v, w_v, wo_v, wr_v, wg_v, wu_v, wd_v, xn_r, res_v, pq_r, m_r, o_r, out_v, sems):
        xn_v, pq_v, m_v, o_v = PB(xn_r), PB(pq_r), PB(m_r), PB(o_r)
        nsem = [0]

        def cp(src, dst):
            c = pltpu.make_async_copy(src, dst, sems.at[nsem[0]])
            nsem[0] += 1
            return c
        NPIECE = S // LNP
        x0_cp = [cp(x_hbm.at[pl.ds(p * LNP, LNP)], x_v.at[pl.ds(p * LNP, LNP)]) for p in range(NPT)]
        xt_cp = [None] + [cp(x_hbm.at[pl.ds(i * TS, TS)], x_v.at[pl.ds(i * TS, TS)]) for i in range(1, NTILE)]
        w_cp = []
        for g in range(G):
            for j in range(3):
                c0 = j * D + g * 128
                w_cp.append(cp(wqkv_hbm.at[:, pl.ds(c0, 128)], w_v.at[:, pl.ds(c0, 128)]))
        wr_cp = cp(wr_hbm, wr_v)
        wo_cp = cp(wo_hbm, wo_v)
        wg_cp = cp(wg_hbm, wg_v)
        wu_cp = cp(wu_hbm, wu_v)
        wd_cp = cp(wd_hbm, wd_v)
        out_cp = {(i, n): cp(out_v.at[pl.ds(i * TS, TS), pl.ds(n * ON, ON)], out_hbm.at[pl.ds(i * TS, TS), pl.ds(n * ON, ON)])
                  for i in range(NTILE) for n in range(NOC)}

        wr_cp.start()
        for p in range(NPT):
            x0_cp[p].start()
        x1pos = cfg.get("x1pos", 12)
        for c in range(x1pos):
            w_cp[c].start()
        xt_cp[1].start()
        for c in range(x1pos, 24):
            w_cp[c].start()
        for i in range(2, NTILE):
            xt_cp[i].start()
        wo_cp.start()
        wg_cp.start()
        wu_cp.start()
        wd_cp.start()

        st = dict(best=None, besti=None)
        piece_iota = lax.broadcasted_iota(jnp.int32, (LNP, 1), 0)

        def ln_piece(p, wr):
            r0 = p * LNP
            rows = pl.ds(r0, LNP)
            x = x_v[rows, :].astype(F32)
            m = jnp.mean(x, axis=-1, keepdims=True)
            xc = x - m
            v = jnp.mean(xc * xc, axis=-1, keepdims=True)
            sd = _rnd(jnp.sqrt(_rnd(_rnd(v) + np.float32(1e-5))))
            xn = (x - _rnd(m)) * (1.0 / sd)
            xnb = xn.astype(BF)
            xn_v.st(r0, 0, xnb)
            res_v[rows, :] = x + xn
            r = _rnd(jnp.sum(xnb.astype(F32) * wr, axis=-1, keepdims=True))
            r = jnp.where(r != r, -jnp.inf, r)
            tm = jnp.max(r, axis=0, keepdims=True)
            ti = jnp.min(jnp.where(r == tm, piece_iota + r0, S), axis=0, keepdims=True)
            if st["best"] is None:
                st["best"], st["besti"] = tm, ti
            else:
                better = tm > st["best"]
                st["best"] = jnp.where(better, tm, st["best"])
                st["besti"] = jnp.where(better, ti, st["besti"])

        wr_cp.wait()
        wr = wr_v[...].astype(F32).reshape(1, D)
        with scope("ln0"):
            for p in range(NPT):
                x0_cp[p].wait()
                ln_piece(p, wr)

        kv = [jnp.zeros((128, 128), F32) for _ in range(G)]
        zacc = [jnp.zeros((8, 128), F32) for _ in range(G)]
        ffn = {}

        def ffn_prep():
            idx = jnp.clip(jnp.min(st["besti"]), 0, S - 1)
            base = pl.multiple_of((idx // 16) * 16, 16)
            ffn["idx"], ffn["base"] = idx, base
            ffn["x16"] = xn_v.ld(base, 16)
            ffn["y"] = jnp.zeros((16, D), F32)
            ffn["h"] = [None] * NFC

        def ffn_gu(c):
            cols = pl.ds(c * FC, FC)
            gt = _dot(ffn["x16"], wg_v[:, cols])
            up = _dot(ffn["x16"], wu_v[:, cols])
            ffn["h"][c] = (gt * jax.nn.sigmoid(gt) * up).astype(BF)

        def ffn_down(c):
            ffn["y"] = ffn["y"] + _dot(ffn["h"][c], wd_v[pl.ds(c * FC, FC), :])

        def ffn_fin():
            gate = jax.nn.sigmoid(st["best"])
            base, idx = ffn["base"], ffn["idx"]
            sel = (lax.broadcasted_iota(jnp.int32, (16, D), 0) + base) == idx
            res_v[pl.ds(base, 16), :] = res_v[pl.ds(base, 16), :] + jnp.where(sel, ffn["y"] * gate, 0.0)

        def proj(i, j, g):
            return _dot(xn_v.ld(i * TS, TS), w_v[:, pl.ds(j * D + g * 128, 128)])

        waited = [0]

        def need_chunk(c):
            if c >= waited[0]:
                hi = 24
                for b_ in bars:
                    if b_ > c or (b_ == c and False):
                        hi = b_
                        break
                hi = max(hi, c + 1)
                for cc in range(waited[0], hi):
                    w_cp[cc].wait()
                if waited[0] < x1pos <= hi or (hi == 24 and waited[0] <= x1pos and False):
                    pass
                waited[0] = hi

        x1_waited = [False]
        for i in range(NTILE):
            if cfg.get("bar2", True):
                if i >= 1 and i + 1 < NTILE:
                    xt_cp[i + 1].wait()
                if i == 2:
                    wo_cp.wait()
            elif i == 1:
                for t in range(2, NTILE):
                    xt_cp[t].wait()
                wo_cp.wait()
            if i == NTILE - 1:
                wg_cp.wait(); wu_cp.wait(); wd_cp.wait()
                if ffn_mode == "tile3":
                    ffn_prep()
            elif i == NTILE - 2 and ffn_mode == "mid":
                pass
            for g in range(G):
                with scope(f"t{i}g{g}"):
                    if i == 0:
                        need_chunk(3 * g)
                    q = proj(i, 0, g)
                    if i == 0:
                        need_chunk(3 * g + 1)
                    k = proj(i, 1, g)
                    pq_v.st(i * TS, g * 128, _phi(q).astype(BF))
                    if i == 0:
                        need_chunk(3 * g + 2)
                    vv = proj(i, 2, g)
                    pk = _phi(k)
                    zacc[g] = zacc[g] + jnp.sum(pk.reshape(TS // 8, 8, 128), axis=0)
                    pkb = pk.astype(BF)
                    if cfg.get("kvmode", "T") == "T":
                        kv[g] = kv[g] + _dot(pkb.T, vv.astype(BF))
                    else:
                        kv[g] = kv[g] + _dot(pkb, vv.astype(BF), TN)
                    if i + 1 < NTILE:
                        lg0 = G - NPT
                        if g >= lg0:
                            if i == 0 and not x1_waited[0]:
                                xt_cp[1].wait()
                                x1_waited[0] = True
                            ln_piece((i + 1) * NPT + (g - lg0), wr)
                    elif ffn_mode == "tile3" and g < NFC:
                        ffn_gu(g)

        ri = lax.broadcasted_iota(jnp.int32, (128, 128), 0) // DH
        ci = lax.broadcasted_iota(jnp.int32, (128, 128), 1) // DH
        mask = ri == ci
        zT = [None] * G

        def mprep(g):
            kvm = jnp.where(mask, kv[g], 0.0).astype(BF)
            m_v.st(g * 128, 0, _dot(kvm, wo_v[pl.ds(g * 128, 128), :]).astype(BF))
            zrow = jnp.sum(zacc[g], axis=0, keepdims=True)
            zT[g] = jnp.where(mask, jnp.broadcast_to(zrow, (128, 128)), 0.0).astype(BF)

        def den_piece(i, g):
            pq = pq_v.ld(i * TS, TS, g * 128, 128)
            den = _dot(pq, zT[g], NT) + 1e-6
            o_v.st(i * TS, g * 128, (pq.astype(F32) / den).astype(BF))

        with scope("mid"):
            if ffn_mode == "mid":
                ffn_prep()
                for c in range(NFC):
                    ffn_gu(c)
            for g in range(G):
                mprep(g)
                if g < NFC:
                    ffn_down(g)
                den_piece(0, g)
            ffn_fin()

        for i in range(NTILE):
            rows = pl.ds(i * TS, TS)
            for n in range(NOC):
                with scope(f"o{i}n{n}"):
                    cols = pl.ds(n * ON, ON)
                    a = _dot(o_v.ld(i * TS, TS), m_v.ld(0, D, n * ON, ON))
                    if i + 1 < NTILE:
                        gpn = G // NOC
                        for g in range(n * gpn, (n + 1) * gpn):
                            den_piece(i + 1, g)
                    out_v[rows, cols] = (res_v[rows, cols] + a).astype(BF)
                    out_cp[(i, n)].start()
        with scope("wait_out"):
            for i in range(NTILE):
                for n in range(NOC):
                    out_cp[(i, n)].wait()

    nsem_total = NPT + NTILE - 1 + 24 + 5 + NTILE * NOC
    wr_shape = cfg.get("wr_shape", (D,))
    pb = (lambda r, c: pltpu.VMEM((r // 2, c), U32)) if packed else (lambda r, c: pltpu.VMEM((r, c), BF))
    scratch = [
        pltpu.VMEM((S, D), BF),
        pltpu.VMEM((D, 3 * D), BF),
        pltpu.VMEM((D, D), BF),
        pltpu.VMEM(wr_shape, BF),
        pltpu.VMEM((D, F), BF),
        pltpu.VMEM((D, F), BF),
        pltpu.VMEM((F, D), BF),
        pb(S, D),
        pltpu.VMEM((S, D), F32),
        pb(S, D),
        pb(D, D),
        pb(S, D),
        pltpu.VMEM((S, D), BF),
        pltpu.SemaphoreType.DMA((nsem_total,)),
    ]

    def fn(A_x, A_wqkv, A_wo, B_x, B_w_r, B_w_gate, B_w_up, B_w_down):
        del B_x
        anyspec = pl.BlockSpec(memory_space=pl.ANY)
        out = pl.pallas_call(
            kernel,
            out_shape=jax.ShapeDtypeStruct((S, D), BF),
            in_specs=[anyspec] * 7,
            out_specs=anyspec,
            scratch_shapes=scratch,
            compiler_params=pltpu.CompilerParams(vmem_limit_bytes=cfg.get("vmem", 100 * 1024 * 1024),
                                                 flags=cfg.get("flags")),
            name=cfg.get("name", "k"),
        )(A_x.reshape(S, D), A_wqkv, A_wo, B_w_r.reshape(wr_shape), B_w_gate, B_w_up, B_w_down)
        return out.reshape(1, S, D)

    return jax.jit(fn)


_KERNEL = None


def pallas_parallel_sum__linear_attn_block__moe_arch_mod__prompt_kernel(
    A_x, A_wqkv, A_wo, B_x, B_w_r, B_w_gate, B_w_up, B_w_down,
):
    fn = make_kernel(dict(name="fused", flags={"XLA_TPU_EVENLY_DISTRIBUTE_CRITICAL_NODES": True}))
    return fn(A_x, A_wqkv, A_wo, B_x, B_w_r, B_w_gate, B_w_up, B_w_down)
```

```python
import contextlib
import numpy as np
import jax
import jax.numpy as jnp
from jax import lax
from jax.experimental import pallas as pl
from jax.experimental.pallas import tpu as pltpu

S, D, H, DH, F = 2048, 1024, 32, 32, 3584
G = D // 128
BF, F32, U32 = jnp.bfloat16, jnp.float32, jnp.uint32
NN = (((1,), (0,)), ((), ()))
NT = (((1,), (1,)), ((), ()))
TN = (((0,), (0,)), ((), ()))


def _dot(a, b, dn=NN):
    return lax.dot_general(a, b, dn, preferred_element_type=F32)


def _rnd(x):
    return x.astype(BF).astype(F32)


def _phi(t):
    return jnp.where(t > 0, t + 1.0, jnp.exp(t)) + 1e-6


class PB:
    def __init__(self, ref):
        self.ref = ref
    def ld(self, r0, nr, c0=0, nc=None):
        nc = self.ref.shape[1] - c0 if nc is None else nc
        if isinstance(r0, int):
            v = self.ref[pl.ds(r0 // 2, nr // 2), pl.ds(c0, nc)]
        else:
            v = self.ref[pl.ds(pl.multiple_of(r0 // 2, 8), nr // 2), pl.ds(c0, nc)]
        return pltpu.bitcast(v, BF)
    def st(self, r0, c0, val):
        nr, nc = val.shape
        self.ref[pl.ds(r0 // 2, nr // 2), pl.ds(c0, nc)] = pltpu.bitcast(val, U32)


def make_kernel(cfg):
    TS = cfg.get("TS", 512)
    NTILE = S // TS
    LNP = cfg.get("LNP", 128)
    LNR = cfg.get("LNR", 32)
    NPT = TS // LNP
    FC = cfg.get("FC", 512)
    NFC = F // FC
    ON = cfg.get("ON", 256)
    NOC = D // ON
    MA = cfg.get("MA", 128)
    MB = cfg.get("MB", 128)
    scopes = cfg.get("scopes", False)
    bars = cfg.get("bars", (1, 2, 4, 8))
    NCH = 16
    NBAR = (1 if cfg.get("bcbar", False) else 0) + ((G // (MB // 128) - 1) if (cfg.get("ffn") == "vpu" and cfg.get("bbar", True)) else 0)
    x1pos = cfg.get("x1pos", 8)

    def scope(name):
        return jax.named_scope(name) if scopes else contextlib.nullcontext()

    def kernel(x_hbm, wqkv_hbm, wo_hbm, wr_hbm, wg_hbm, wu_hbm, wd_hbm, out_hbm,
               x_v, w_v, wo_v, wr_v, wg_v, wu_v, wd_v, xn_r, res_v, wT_r, pqT_r, pkT_r, m_r, o_r, out_v, xb_v, hb_v, bar_v, p_r, sems):
        p_v = PB(p_r)
        xn_v, wT_v, pqT_v, pkT_v, m_v, o_v = PB(xn_r), PB(wT_r), PB(pqT_r), PB(pkT_r), PB(m_r), PB(o_r)
        nsem = [0]

        def cp(src, dst):
            c = pltpu.make_async_copy(src, dst, sems.at[nsem[0]])
            nsem[0] += 1
            return c
        x0_cp = [cp(x_hbm.at[pl.ds(p * LNP, LNP)], x_v.at[pl.ds(p * LNP, LNP)]) for p in range(NPT)]
        xt_cp = [None] + [cp(x_hbm.at[pl.ds(i * TS, TS)], x_v.at[pl.ds(i * TS, TS)]) for i in range(1, NTILE)]
        w_cp = []
        for g in range(G):
            for j in range(2):
                c0 = j * D + g * 128
                w_cp.append(cp(wqkv_hbm.at[:, pl.ds(c0, 128)], w_v.at[:, pl.ds(c0, 128)]))
        wv_cp = cp(wqkv_hbm.at[:, pl.ds(2 * D, D)], w_v.at[:, pl.ds(2 * D, D)])
        wr_cp = cp(wr_hbm, wr_v)
        wo_cp = cp(wo_hbm, wo_v)
        bar_cp = [cp(x_hbm.at[pl.ds(0, 16)], bar_v.at[pl.ds(16 * k_, 16)]) for k_ in range(NBAR)]
        wg_cp = cp(wg_hbm, wg_v)
        wu_cp = cp(wu_hbm, wu_v)
        wd_cp = cp(wd_hbm, wd_v)
        out_cp = {(i, n): cp(out_v.at[pl.ds(i * TS, TS), pl.ds(n * ON, ON)], out_hbm.at[pl.ds(i * TS, TS), pl.ds(n * ON, ON)])
                  for i in range(NTILE) for n in range(NOC)}

        wr_cp.start()
        for c_ in bar_cp:
            c_.start()
        bar_i = [0]

        def barrier():
            bar_cp[bar_i[0]].wait()
            bar_i[0] += 1

        for p in range(NPT):
            x0_cp[p].start()
        for c in range(x1pos):
            w_cp[c].start()
        xt_cp[1].start()
        for c in range(x1pos, NCH):
            w_cp[c].start()
        for i in range(2, NTILE):
            xt_cp[i].start()
        wv_cp.start()
        wo_cp.start()
        wg_cp.start()
        wu_cp.start()
        wd_cp.start()

        st = dict(best=None, besti=None)
        grp_iota = lax.broadcasted_iota(jnp.int32, (LNR, 1), 0)

        def ln_group(r0, wr):
            rows = pl.ds(r0, LNR)
            x = x_v[rows, :].astype(F32)
            m = jnp.mean(x, axis=-1, keepdims=True)
            mb = _rnd(m)
            xc = x - mb
            dm = m - mb
            v = jnp.mean(xc * xc, axis=-1, keepdims=True) - dm * dm
            sd = _rnd(jnp.sqrt(_rnd(_rnd(v) + np.float32(1e-5))))
            xn = xc * (1.0 / sd)
            xnb = xn.astype(BF)
            xn_v.st(r0, 0, xnb)
            res_v[rows, :] = x + xn
            r = _rnd(jnp.sum(xnb.astype(F32) * wr, axis=-1, keepdims=True))
            r = jnp.where(r != r, -jnp.inf, r)
            ri = grp_iota + r0
            if st["best"] is None:
                st["best"], st["besti"] = r, ri
            else:
                better = r > st["best"]
                st["best"] = jnp.where(better, r, st["best"])
                st["besti"] = jnp.where(better, ri, st["besti"])

        def ln_rows(r0, n):
            for k in range(n // LNR):
                ln_group(r0 + k * LNR, wr)

        wr_cp.wait()
        wr = wr_v[...].astype(F32).reshape(1, D)
        with scope("ln0"):
            for p in range(NPT):
                x0_cp[p].wait()
                ln_rows(p * LNP, LNP)

        zacc = [jnp.zeros((128, 128), F32) for _ in range(G)]
        ffn = {}

        def ffn_prep():
            best, besti = st["best"], st["besti"]
            bm = jnp.max(best, axis=0, keepdims=True)
            bi = jnp.min(jnp.where(best == bm, besti, S), axis=0, keepdims=True)
            idx = jnp.clip(jnp.min(bi), 0, S - 1)
            base = pl.multiple_of((idx // 16) * 16, 16)
            ffn["idx"], ffn["base"], ffn["rmax"] = idx, base, bm
            ffn["x16"] = xn_v.ld(base, 16)
            ffn["y"] = jnp.zeros((16, D), F32)
            ffn["h"] = [None] * NFC

        def ffn_gu(c):
            cols = pl.ds(c * FC, FC)
            gt = _dot(ffn["x16"], wg_v[:, cols])
            up = _dot(ffn["x16"], wu_v[:, cols])
            ffn["h"][c] = (gt * jax.nn.sigmoid(gt) * up).astype(BF)

        def ffn_down(c):
            ffn["y"] = ffn["y"] + _dot(ffn["h"][c], wd_v[pl.ds(c * FC, FC), :])

        def ffn_fin():
            gate = jax.nn.sigmoid(ffn["rmax"])
            base, idx = ffn["base"], ffn["idx"]
            sel = (lax.broadcasted_iota(jnp.int32, (16, D), 0) + base) == idx
            res_v[pl.ds(base, 16), :] = res_v[pl.ds(base, 16), :] + jnp.where(sel, ffn["y"] * gate, 0.0)

        KB = cfg.get("KB", 16)
        def vffn_prep():
            best, besti = st["best"], st["besti"]
            bm = jnp.max(best, axis=0, keepdims=True)
            bi = jnp.min(jnp.where(best == bm, besti, S), axis=0, keepdims=True)
            idx = jnp.clip(jnp.min(bi), 0, S - 1)
            base = pl.multiple_of((idx // 16) * 16, 16)
            ffn["idx"], ffn["base"], ffn["rmax"] = idx, base, bm
            x16 = xn_v.ld(base, 16).astype(F32)
            sel = (lax.broadcasted_iota(jnp.int32, (16, D), 0) + base) == idx
            xs = jnp.sum(jnp.where(sel, x16, 0.0), axis=0, keepdims=True)
            for b_ in range(D // 128):
                blk = jnp.broadcast_to(xs[:, b_ * 128:(b_ + 1) * 128], (128, 128))
                xb_v[pl.ds(b_ * 128, 128), :] = blk.T
            ffn["g"] = {}

        def vffn_gu(c, k0, k1, first, last):
            nl = FC // 128
            if first:
                ag = [jnp.zeros((8, 128), F32) for _ in range(nl)]
                au = [jnp.zeros((8, 128), F32) for _ in range(nl)]
            else:
                ag, au = ffn["g"][c]
            for kb in range(k0, k1, 8):
                xk = xb_v[pl.ds(kb, 8), :]
                for l2 in range(nl // 2):
                    cols = pl.ds(c * FC + l2 * 256, 256)
                    wg = wg_v[pl.ds(kb, 8), cols].astype(F32)
                    wu = wu_v[pl.ds(kb, 8), cols].astype(F32)
                    for t in range(2):
                        ag[2 * l2 + t] = ag[2 * l2 + t] + wg[:, t * 128:(t + 1) * 128] * xk
                        au[2 * l2 + t] = au[2 * l2 + t] + wu[:, t * 128:(t + 1) * 128] * xk
            if last:
                for b_ in range(nl):
                    gt = jnp.sum(ag[b_], axis=0, keepdims=True)
                    up = jnp.sum(au[b_], axis=0, keepdims=True)
                    h = gt * jax.nn.sigmoid(gt) * up
                    if cfg.get("hround", True):
                        h = _rnd(h)
                    hb_v[pl.ds(c * FC + b_ * 128, 128), :] = jnp.broadcast_to(h, (128, 128)).T
            else:
                ffn["g"][c] = (ag, au)

        def vffn_down(f0, f1, first):
            nl = D // 128
            if first:
                ay = [jnp.zeros((8, 128), F32) for _ in range(nl)]
            else:
                ay = ffn["ay"]
            for fb in range(f0, f1, 8):
                hk = hb_v[pl.ds(fb, 8), :]
                for l2 in range(nl // 2):
                    w = wd_v[pl.ds(fb, 8), pl.ds(l2 * 256, 256)].astype(F32)
                    for t in range(2):
                        ay[2 * l2 + t] = ay[2 * l2 + t] + w[:, t * 128:(t + 1) * 128] * hk
            ffn["ay"] = ay

        def vffn_fin():
            y = jnp.concatenate([jnp.sum(a_, axis=0, keepdims=True) for a_ in ffn["ay"]], axis=1)
            gate = jax.nn.sigmoid(ffn["rmax"])
            base, idx = ffn["base"], ffn["idx"]
            sel = (lax.broadcasted_iota(jnp.int32, (16, D), 0) + base) == idx
            res_v[pl.ds(base, 16), :] = res_v[pl.ds(base, 16), :] + jnp.where(sel, y * gate, 0.0)

        waited = [0]
        x1_waited = [False]

        def need_chunk(c):
            if c >= waited[0]:
                hi = NCH
                for b_ in bars:
                    if b_ > c:
                        hi = b_
                        break
                for cc in range(waited[0], hi):
                    w_cp[cc].wait()
                if hi >= x1pos and not x1_waited[0]:
                    xt_cp[1].wait()
                    x1_waited[0] = True
                for cc in range(waited[0], hi):
                    g, j = cc // 2, cc % 2
                    c0 = j * D + g * 128
                    wT_v.st(j * D + g * 128, 0, w_v[:, pl.ds(c0, 128)].T)
                waited[0] = hi

        def projT(i, j, r0, nr):
            return _dot(wT_v.ld(j * D + r0, nr), xn_v.ld(i * TS, TS), NT)

        gpd = MA // 128
        for i in range(NTILE):
            if cfg.get("barmode", "tile") in ("tile", "tile3"):
                if i >= 1 and i + 1 < NTILE:
                    xt_cp[i + 1].wait()
                if i == NTILE - 1 and cfg.get("barmode") == "tile3":
                    wv_cp.wait()
                    wo_cp.wait()
            elif i == 1:
                for t in range(2, NTILE):
                    xt_cp[t].wait()
            for gb in range(G // gpd):
                with scope(f"a{i}"):
                    if i == 0:
                        need_chunk(2 * (gb * gpd + gpd - 1) + 0)
                    qT = projT(i, 0, gb * MA, MA)
                    if i == 0:
                        need_chunk(2 * (gb * gpd + gpd - 1) + 1)
                    kT = projT(i, 1, gb * MA, MA)
                    pqT_v.st(gb * MA, i * TS, _phi(qT).astype(BF))
                    pk = _phi(kT)
                    for t in range(gpd):
                        blk = pk[t * 128:(t + 1) * 128]
                        acc = zacc[gb * gpd + t]
                        for n in range(TS // 128):
                            acc = acc + blk[:, n * 128:(n + 1) * 128]
                        zacc[gb * gpd + t] = acc
                    pkT_v.st(gb * MA, i * TS, pk.astype(BF))
                    if i + 1 < NTILE:
                        nb = G // gpd
                        rows_per = TS // nb
                        if i == 0:
                            if gb >= nb // 2:
                                assert x1_waited[0]
                                ln_rows((i + 1) * TS + (gb - nb // 2) * 2 * rows_per, 2 * rows_per)
                        elif cfg.get("lnspread", True):
                            ln_rows((i + 1) * TS + gb * rows_per, rows_per)
                        elif gb == nb - 1:
                            ln_rows((i + 1) * TS, TS)

        ri = lax.broadcasted_iota(jnp.int32, (128, 128), 0) // DH
        ci = lax.broadcasted_iota(jnp.int32, (128, 128), 1) // DH
        mask = ri == ci
        zcol = [None] * G

        def den_piece(i, g):
            p = pqT_v.ld(g * 128, 128, i * TS, TS).astype(F32)
            zb = jnp.concatenate([zcol[g]] * (TS // 128), axis=1)
            p4 = p.reshape(4, DH, TS)
            den = jnp.sum(p4 * zb.reshape(4, DH, TS), axis=1, keepdims=True) + 1e-6
            o = (p4 * (1.0 / den)).reshape(128, TS).astype(BF)
            o_v.st(i * TS, g * 128, o.T)

        with scope("b"):
            if cfg.get("barmode", "tile") != "tile3":
                wv_cp.wait()
                wo_cp.wait()
            if cfg.get("ffnpipe", 0) == 0:
                wg_cp.wait(); wu_cp.wait(); wd_cp.wait()
            if cfg.get("ffn") == "vpu":
                vffn_prep()
            else:
                ffn_prep()
            for g in range(G):
                zcol[g] = jnp.broadcast_to(jnp.sum(zacc[g], axis=1, keepdims=True), (128, 128))
            gpb = MB // 128
            NB = G // gpb
            Ps = [None] * NB

            def p_blk(gb):
                Ps[gb] = _dot(pkT_v.ld(gb * MB, MB), xn_v.ld(0, S)).astype(BF)

            def kvm_blk(gb):
                for t in range(gpb):
                    g = gb * gpb + t
                    kv = _dot(Ps[gb][t * 128:(t + 1) * 128], w_v[:, pl.ds(2 * D + g * 128, 128)])
                    kvm = jnp.where(mask, kv, 0.0).astype(BF)
                    m_v.st(g * 128, 0, _dot(kvm, wo_v[pl.ds(g * 128, 128), :]).astype(BF))

            def kvm_blk2(gb):
                for t in range(gpb):
                    g = gb * gpb + t
                    kv = _dot(p_v.ld(g * 128, 128), w_v[:, pl.ds(2 * D + g * 128, 128)])
                    kvm = jnp.where(mask, kv, 0.0).astype(BF)
                    m_v.st(g * 128, 0, _dot(kvm, wo_v[pl.ds(g * 128, 128), :]).astype(BF))

            fpipe = cfg.get("ffnpipe", 0)
            if cfg.get("ffn") == "vpu":
                tasks = []
                for c in range(NFC):
                    tasks.append((FC * 2 * 3.0, (lambda c=c: vffn_gu(c, 0, D, True, True))))
                nd = cfg.get("dsplit", 14)
                fbs = [(dd * (F // 8) // nd) * 8 for dd in range(nd + 1)]
                for dd in range(nd):
                    tasks.append(((fbs[dd + 1] - fbs[dd]) * 3.0, (lambda dd=dd: vffn_down(fbs[dd], fbs[dd + 1], dd == 0))))
                tot = sum(c_ for c_, _ in tasks)
                nreg = NB
                bounds = cfg.get("fbounds", None)
                ti = 0
                cum = 0.0
                dpr = G // nreg
                for r in range(nreg):
                    if r > 0 and cfg.get("bbar", True):
                        barrier()
                    p_v.st(r * MB, 0, _dot(pkT_v.ld(r * MB, MB), xn_v.ld(0, S)).astype(BF))
                    if r > 0:
                        kvm_blk2(r - 1)
                    lim = tot * (r + 1) / nreg if bounds is None else tot * bounds[r]
                    while ti < len(tasks) and cum + tasks[ti][0] * 0.5 <= lim:
                        cum += tasks[ti][0]
                        tasks[ti][1](); ti += 1
                    for g in range(r * dpr, (r + 1) * dpr):
                        den_piece(0, g)
                kvm_blk2(nreg - 1)
                while ti < len(tasks):
                    tasks[ti][1](); ti += 1
                vffn_fin()
            elif fpipe == 0:
                p_blk(0)
                for gb in range(NB):
                    if gb + 1 < NB:
                        p_blk(gb + 1)
                    kvm_blk(gb)
                    for g in range(gb * gpb, (gb + 1) * gpb):
                        if g < NFC:
                            ffn_gu(g)
                        den_piece(0, g)
                for c in range(NFC):
                    ffn_down(c)
                ffn_fin()
            else:
                p_blk(0)
                for gb in range(NB - 1):
                    p_blk(gb + 1)
                    kvm_blk(gb)
                    for g in range(gb * gpb, (gb + 1) * gpb):
                        den_piece(0, g)
                    if gb == NB - 2 - (fpipe - 1):
                        wg_cp.wait(); wu_cp.wait(); wd_cp.wait()
                for c in range(NFC):
                    ffn_gu(c)
                kvm_blk(NB - 1)
                for g in range((NB - 1) * gpb, G):
                    den_piece(0, g)
                for c in range(NFC):
                    ffn_down(c)
                ffn_fin()

        if cfg.get("bcbar", False):
            barrier()
        for i in range(NTILE):
            rows = pl.ds(i * TS, TS)
            for n in range(NOC):
                with scope(f"o{i}"):
                    cols = pl.ds(n * ON, ON)
                    a = _dot(o_v.ld(i * TS, TS), m_v.ld(0, D, n * ON, ON))
                    if i + 1 < NTILE:
                        gpn = G // NOC
                        for g in range(n * gpn, (n + 1) * gpn):
                            den_piece(i + 1, g)
                    out_v[rows, cols] = (res_v[rows, cols] + a).astype(BF)
                    out_cp[(i, n)].start()
        with scope("wait_out"):
            for i in range(NTILE):
                for n in range(NOC):
                    out_cp[(i, n)].wait()

    nsem_total = NPT + NTILE - 1 + NCH + 6 + NTILE * NOC + NBAR
    pb = lambda r, c: pltpu.VMEM((r // 2, c), U32)
    scratch = [
        pltpu.VMEM((S, D), BF),
        pltpu.VMEM((D, 3 * D), BF),
        pltpu.VMEM((D, D), BF),
        pltpu.VMEM((D,), BF),
        pltpu.VMEM((D, F), BF),
        pltpu.VMEM((D, F), BF),
        pltpu.VMEM((F, D), BF),
        pb(S, D),
        pltpu.VMEM((S, D), F32),
        pb(2 * D, D),
        pb(D, S),
        pb(D, S),
        pb(D, D),
        pb(S, D),
        pltpu.VMEM((S, D), BF),
        pltpu.VMEM((D, 128), F32),
        pltpu.VMEM((F, 128), F32),
        pltpu.VMEM((16 * max(NBAR, 1), D), BF),
        pb(D, D),
        pltpu.SemaphoreType.DMA((nsem_total,)),
    ]

    def fn(A_x, A_wqkv, A_wo, B_x, B_w_r, B_w_gate, B_w_up, B_w_down):
        del B_x
        anyspec = pl.BlockSpec(memory_space=pl.ANY)
        out = pl.pallas_call(
            kernel,
            out_shape=jax.ShapeDtypeStruct((S, D), BF),
            in_specs=[anyspec] * 7,
            out_specs=anyspec,
            scratch_shapes=scratch,
            compiler_params=pltpu.CompilerParams(vmem_limit_bytes=cfg.get("vmem", 110 * 1024 * 1024),
                                                 flags=cfg.get("flags")),
            name=cfg.get("name", "k"),
        )(A_x.reshape(S, D), A_wqkv, A_wo, B_w_r, B_w_gate, B_w_up, B_w_down)
        return out.reshape(1, S, D)

    return jax.jit(fn)


def pallas_parallel_sum__linear_attn_block__moe_arch_mod__prompt_kernel(
    A_x, A_wqkv, A_wo, B_x, B_w_r, B_w_gate, B_w_up, B_w_down,
):
    fn = make_kernel(dict(name='fused', MA=256, MB=256, flags={'XLA_TPU_EVENLY_DISTRIBUTE_CRITICAL_NODES': True}, barmode='tile3', bcbar=False))
    return fn(A_x, A_wqkv, A_wo, B_x, B_w_r, B_w_gate, B_w_up, B_w_down)
```

```python
import contextlib
import numpy as np
import jax
import jax.numpy as jnp
from jax import lax
from jax.experimental import pallas as pl
from jax.experimental.pallas import tpu as pltpu

S, D, H, DH, F = 2048, 1024, 32, 32, 3584
G = D // 128
BF, F32, U32 = jnp.bfloat16, jnp.float32, jnp.uint32
NN = (((1,), (0,)), ((), ()))
NT = (((1,), (1,)), ((), ()))


def _dot(a, b, dn=NN):
    return lax.dot_general(a, b, dn, preferred_element_type=F32)


def _rnd(x):
    return x.astype(BF).astype(F32)


def _phi(t):
    return jnp.where(t > 0, t + 1.0, jnp.exp(t)) + 1e-6


class PB:
    def __init__(self, ref):
        self.ref = ref
    def ld(self, r0, nr, c0=0, nc=None):
        nc = self.ref.shape[1] - c0 if nc is None else nc
        if isinstance(r0, int):
            v = self.ref[pl.ds(r0 // 2, nr // 2), pl.ds(c0, nc)]
        else:
            v = self.ref[pl.ds(pl.multiple_of(r0 // 2, 8), nr // 2), pl.ds(c0, nc)]
        return pltpu.bitcast(v, BF)
    def st(self, r0, c0, val):
        nr, nc = val.shape
        self.ref[pl.ds(r0 // 2, nr // 2), pl.ds(c0, nc)] = pltpu.bitcast(val, U32)


def make_kernel(cfg):
    TS = 512
    NTILE = S // TS
    LNP = cfg.get("LNP", 128)
    LNR = cfg.get("LNR", 32)
    NPT = TS // LNP
    FC = cfg.get("FC", 512)
    NFC = F // FC
    ON = cfg.get("ON", 256)
    NOC = D // ON
    MA = cfg.get("MA", 512)
    MB = cfg.get("MB", 256)
    segs = cfg.get("segs", (1, 2, 4, 5, 4))
    NCH = 16
    assert sum(segs) == NCH
    x1pos = cfg.get("x1pos", NCH)
    x1seg = cfg.get("x1seg", len(segs) - 1)
    scopes = cfg.get("scopes", False)
    nbar = cfg.get("nbar", 0)

    def scope(name):
        return jax.named_scope(name) if scopes else contextlib.nullcontext()

    def kernel(x_hbm, wqkv_hbm, wo_hbm, wr_hbm, wg_hbm, wu_hbm, wd_hbm, out_hbm,
               x_v, w_v, wo_v, wr_v, wg_v, wu_v, wd_v, xn_r, res_v, wT_r, pqT_r, pkT_r, m_r, o_r, p_r, z_v, out_v, xb_v, hb_v, bar_v, sems):
        xn_v, wT_v, pqT_v, pkT_v, m_v, o_v, p_v = (PB(r) for r in (xn_r, wT_r, pqT_r, pkT_r, m_r, o_r, p_r))
        nsem = [0]

        def cp(src, dst):
            c = pltpu.make_async_copy(src, dst, sems.at[nsem[0]])
            nsem[0] += 1
            return c
        x0_cp = [cp(x_hbm.at[pl.ds(p * LNP, LNP)], x_v.at[pl.ds(p * LNP, LNP)]) for p in range(NPT)]
        xt_cp = [None] + [cp(x_hbm.at[pl.ds(i * TS, TS)], x_v.at[pl.ds(i * TS, TS)]) for i in range(1, NTILE)]
        w_cp = []
        for c in range(NCH):
            c0 = (c % 2) * D + (c // 2) * 128
            w_cp.append(cp(wqkv_hbm.at[:, pl.ds(c0, 128)], w_v.at[:, pl.ds(c0, 128)]))
        wv_cp = cp(wqkv_hbm.at[:, pl.ds(2 * D, D)], w_v.at[:, pl.ds(2 * D, D)])
        wr_cp = cp(wr_hbm, wr_v)
        wo_cp = cp(wo_hbm, wo_v)
        bar_cp = cp(x_hbm.at[pl.ds(0, 16)], bar_v) if cfg.get("bcbar", False) else None
        wg_cp = cp(wg_hbm, wg_v)
        wu_cp = cp(wu_hbm, wu_v)
        wd_cp = cp(wd_hbm, wd_v)
        out_cp = {(i, n): cp(out_v.at[pl.ds(i * TS, TS), pl.ds(n * ON, ON)], out_hbm.at[pl.ds(i * TS, TS), pl.ds(n * ON, ON)])
                  for i in range(NTILE) for n in range(NOC)}

        for p in range(NPT):
            x0_cp[p].start()
            if p == 0:
                wr_cp.start()
        for c in range(x1pos):
            w_cp[c].start()
        xt_cp[1].start()
        for c in range(x1pos, NCH):
            w_cp[c].start()
        for i in range(2, NTILE):
            xt_cp[i].start()
        wv_cp.start()
        if bar_cp is not None:
            bar_cp.start()
        wo_cp.start()
        wg_cp.start()
        wu_cp.start()
        wd_cp.start()

        st = dict(best=None, besti=None)
        grp_iota = lax.broadcasted_iota(jnp.int32, (LNR, 1), 0)

        def ln_xn_group(r0):
            x = x_v[pl.ds(r0, LNR), :].astype(F32)
            m = jnp.mean(x, axis=-1, keepdims=True)
            mb = _rnd(m)
            xc = x - mb
            dm = m - mb
            v = jnp.mean(xc * xc, axis=-1, keepdims=True) - dm * dm
            sd = _rnd(jnp.sqrt(_rnd(_rnd(v) + np.float32(1e-5))))
            xn_v.st(r0, 0, (xc * (1.0 / sd)).astype(BF))

        def ln_xn(r0, n):
            for k in range(n // LNR):
                ln_xn_group(r0 + k * LNR)

        def ln_post_group(r0, wr):
            x = x_v[pl.ds(r0, LNR), :].astype(F32)
            xn = xn_v.ld(r0, LNR).astype(F32)
            res_v[pl.ds(r0, LNR), :] = x + xn
            r = _rnd(jnp.sum(xn * wr, axis=-1, keepdims=True))
            r = jnp.where(r != r, -jnp.inf, r)
            ri = grp_iota + r0
            if st["best"] is None:
                st["best"], st["besti"] = r, ri
            else:
                better = r > st["best"]
                st["best"] = jnp.where(better, r, st["best"])
                st["besti"] = jnp.where(better, ri, st["besti"])

        def ln_post(r0, n):
            wr = st["wr"]
            for k in range(n // LNR):
                ln_post_group(r0 + k * LNR, wr)

        def ln_full(r0, n):
            wr = st["wr"]
            for k in range(n // LNR):
                rr = r0 + k * LNR
                x = x_v[pl.ds(rr, LNR), :].astype(F32)
                m = jnp.mean(x, axis=-1, keepdims=True)
                mb = _rnd(m)
                xc = x - mb
                dm = m - mb
                v = jnp.mean(xc * xc, axis=-1, keepdims=True) - dm * dm
                sd = _rnd(jnp.sqrt(_rnd(_rnd(v) + np.float32(1e-5))))
                xnb = (xc * (1.0 / sd)).astype(BF)
                xn_v.st(rr, 0, xnb)
                xn = xnb.astype(F32)
                res_v[pl.ds(rr, LNR), :] = x + xn
                r = _rnd(jnp.sum(xn * wr, axis=-1, keepdims=True))
                r = jnp.where(r != r, -jnp.inf, r)
                ri = grp_iota + rr
                if st["best"] is None:
                    st["best"], st["besti"] = r, ri
                else:
                    better = r > st["best"]
                    st["best"] = jnp.where(better, r, st["best"])
                    st["besti"] = jnp.where(better, ri, st["besti"])

        with scope("ln0"):
            for p in range(NPT):
                x0_cp[p].wait()
                if p == NPT - 1:
                    wr_cp.wait()
                    st["wr"] = wr_v[...].astype(F32).reshape(1, D)
                ln_xn(p * LNP, LNP)

        def proj_post(i, j, r0, nr, t):
            p = _phi(t)
            if j == 0:
                pqT_v.st(r0, i * TS, p.astype(BF))
            else:
                zs = p[:, 0:128]
                for n in range(1, TS // 128):
                    zs = zs + p[:, n * 128:(n + 1) * 128]
                if i == 0:
                    z_v[pl.ds(r0, nr), :] = zs
                else:
                    z_v[pl.ds(r0, nr), :] = z_v[pl.ds(r0, nr), :] + zs
                pkT_v.st(r0, i * TS, p.astype(BF))

        def projT(i, j, r0, nr):
            return _dot(wT_v.ld(j * D + r0, nr), xn_v.ld(i * TS, TS), NT)

        def spread(fn, r0, n, k, nk):
            ng = n // LNR
            a, b = k * ng // nk, (k + 1) * ng // nk
            if b > a:
                fn(r0 + a * LNR, (b - a) * LNR)

        c0_ = 0
        for si, sn in enumerate(segs):
            with scope(f"w{si}"):
                for c in range(c0_, c0_ + sn):
                    w_cp[c].wait()
                if si == x1seg:
                    xt_cp[1].wait()
            with scope(f"a0s{si}"):
                for c in range(c0_, c0_ + sn):
                    g, j = c // 2, c % 2
                    wT_v.st(j * D + g * 128, 0, w_v[:, pl.ds(j * D + g * 128, 128)].T)
                for k, c in enumerate(range(c0_, c0_ + sn)):
                    g, j = c // 2, c % 2
                    proj_post(0, j, g * 128, 128, projT(0, j, g * 128, 128))
                    if si == x1seg - cfg.get("post0off", 1):
                        spread(ln_post, 0, TS, k, sn)
                    if si == x1seg:
                        spread(ln_xn, TS, TS, k, sn)
            c0_ += sn

        nd = 2 * (D // MA)
        for i in range(1, NTILE):
            with scope(f"wt{i}"):
                if i + 1 < NTILE:
                    xt_cp[i + 1].wait()
                if i == NTILE - 1:
                    wv_cp.wait()
                    wo_cp.wait()
                    if cfg.get("guwait", "b") == "t3":
                        wg_cp.wait(); wu_cp.wait()
            with scope(f"a{i}"):
                k = 0
                for rb in range(D // MA):
                    for j in range(2):
                        proj_post(i, j, rb * MA, MA, projT(i, j, rb * MA, MA))
                        if cfg.get("lnmode", "split") == "split":
                            if i + 1 < NTILE:
                                spread(ln_xn, (i + 1) * TS, TS, k, nd)
                            spread(ln_post, i * TS, TS, k, nd)
                        k += 1

        ri = lax.broadcasted_iota(jnp.int32, (128, 128), 0) // DH
        ci = lax.broadcasted_iota(jnp.int32, (128, 128), 1) // DH
        mask = ri == ci
        zcol = [None] * G
        ffn = {}

        def ffn_prep():
            best, besti = st["best"], st["besti"]
            bm = jnp.max(best, axis=0, keepdims=True)
            bi = jnp.min(jnp.where(best == bm, besti, S), axis=0, keepdims=True)
            idx = jnp.clip(jnp.min(bi), 0, S - 1)
            base = pl.multiple_of((idx // 16) * 16, 16)
            ffn["idx"], ffn["base"], ffn["rmax"] = idx, base, bm
            ffn["x16"] = xn_v.ld(base, 16)
            ffn["y"] = jnp.zeros((16, D), F32)
            ffn["h"] = [None] * NFC

        def ffn_gu(c):
            cols = pl.ds(c * FC, FC)
            gt = _dot(ffn["x16"], wg_v[:, cols])
            up = _dot(ffn["x16"], wu_v[:, cols])
            ffn["h"][c] = (gt * jax.nn.sigmoid(gt) * up).astype(BF)

        def ffn_down(c):
            ffn["y"] = ffn["y"] + _dot(ffn["h"][c], wd_v[pl.ds(c * FC, FC), :])

        def ffn_fin():
            gate = jax.nn.sigmoid(ffn["rmax"])
            base, idx = ffn["base"], ffn["idx"]
            sel = (lax.broadcasted_iota(jnp.int32, (16, D), 0) + base) == idx
            res_v[pl.ds(base, 16), :] = res_v[pl.ds(base, 16), :] + jnp.where(sel, ffn["y"] * gate, 0.0)

        def vffn_prep():
            best, besti = st["best"], st["besti"]
            bm = jnp.max(best, axis=0, keepdims=True)
            bi = jnp.min(jnp.where(best == bm, besti, S), axis=0, keepdims=True)
            idx = jnp.clip(jnp.min(bi), 0, S - 1)
            base = pl.multiple_of((idx // 16) * 16, 16)
            ffn["idx"], ffn["base"], ffn["rmax"] = idx, base, bm
            x16 = xn_v.ld(base, 16).astype(F32)
            sel = (lax.broadcasted_iota(jnp.int32, (16, D), 0) + base) == idx
            xs = jnp.sum(jnp.where(sel, x16, 0.0), axis=0, keepdims=True)
            for b_ in range(D // 128):
                xb_v[pl.ds(b_ * 128, 128), :] = jnp.broadcast_to(xs[:, b_ * 128:(b_ + 1) * 128], (128, 128)).T

        def vmatvec(w_list, col_ref, k0, k1, c0, nc):
            nl = nc // 128
            acc = [[None] * nl for _ in w_list]
            for kb in range(k0, k1, 8):
                xk = col_ref[pl.ds(kb, 8), :]
                for l2 in range(nl // 2):
                    cols = pl.ds(c0 + l2 * 256, 256)
                    for wi, w_ref in enumerate(w_list):
                        w = w_ref[pl.ds(kb, 8), cols].astype(F32)
                        for t in range(2):
                            pr = w[:, t * 128:(t + 1) * 128] * xk
                            a_ = acc[wi][2 * l2 + t]
                            acc[wi][2 * l2 + t] = pr if a_ is None else a_ + pr
            return acc

        def vffn_gu(c):
            ag, au = vmatvec([wg_v, wu_v], xb_v, 0, D, c * FC, FC)
            for b_ in range(FC // 128):
                gt = jnp.sum(ag[b_], axis=0, keepdims=True)
                up = jnp.sum(au[b_], axis=0, keepdims=True)
                h = gt * jax.nn.sigmoid(gt) * up
                hb_v[pl.ds(c * FC + b_ * 128, 128), :] = jnp.broadcast_to(h, (128, 128)).T

        def vffn_down(c):
            (ay,) = vmatvec([wd_v], hb_v, c * FC, (c + 1) * FC, 0, D)
            if ffn.get("ay") is None:
                ffn["ay"] = ay
            else:
                ffn["ay"] = [a_ + b_ for a_, b_ in zip(ffn["ay"], ay)]

        def vffn_fin():
            y = jnp.concatenate([jnp.sum(a_, axis=0, keepdims=True) for a_ in ffn["ay"]], axis=1)
            gate = jax.nn.sigmoid(ffn["rmax"])
            base, idx = ffn["base"], ffn["idx"]
            sel = (lax.broadcasted_iota(jnp.int32, (16, D), 0) + base) == idx
            res_v[pl.ds(base, 16), :] = res_v[pl.ds(base, 16), :] + jnp.where(sel, y * gate, 0.0)

        if cfg.get("ffn") == "vpu":
            ffn_prep, ffn_gu, ffn_down, ffn_fin = vffn_prep, vffn_gu, vffn_down, vffn_fin

        def den_piece(i, g):
            p = pqT_v.ld(g * 128, 128, i * TS, TS).astype(F32)
            zb = jnp.concatenate([zcol[g]] * (TS // 128), axis=1)
            p4 = p.reshape(4, DH, TS)
            den = jnp.sum(p4 * zb.reshape(4, DH, TS), axis=1, keepdims=True) + 1e-6
            o = (p4 * (1.0 / den)).reshape(128, TS).astype(BF)
            o_v.st(i * TS, g * 128, o.T)

        def p_blk(gb):
            p_v.st(gb * MB, 0, _dot(pkT_v.ld(gb * MB, MB), xn_v.ld(0, S)).astype(BF))

        def kvm_blk(gb):
            for g in range(gb * MB // 128, (gb + 1) * MB // 128):
                kv = _dot(p_v.ld(g * 128, 128), w_v[:, pl.ds(2 * D + g * 128, 128)])
                kvm = jnp.where(mask, kv, 0.0).astype(BF)
                m_v.st(g * 128, 0, _dot(kvm, wo_v[pl.ds(g * 128, 128), :]).astype(BF))

        with scope("b"):
            fwait = cfg.get("fwait", 1)
            split = cfg.get("wdwait", None) is not None
            if split:
                if cfg.get("guwait", "b") == "b":
                    wg_cp.wait(); wu_cp.wait()
            elif fwait == 0:
                wg_cp.wait(); wu_cp.wait(); wd_cp.wait()
            ffn_prep()
            for g in range(G):
                zcol[g] = jnp.broadcast_to(jnp.sum(z_v[pl.ds(g * 128, 128), :], axis=1, keepdims=True), (128, 128))
            NB = D // MB
            gpb = MB // 128
            fsched = cfg.get("fsched", None)
            if fsched is None and split:
                w_ = cfg["wdwait"]
                fsched = []
                for gb in range(NB):
                    if gb < w_:
                        fsched.append((list(range(gb * NFC // w_, (gb + 1) * NFC // w_)), []))
                    else:
                        k_, n_ = gb - w_, NB - w_
                        fsched.append(([], list(range(k_ * NFC // n_, (k_ + 1) * NFC // n_))))
            if fsched is None:
                nact = NB - fwait
                per = -(-NFC // nact)
                fsched = [([], []) for _ in range(fwait)]
                for k_ in range(nact):
                    fsched.append((list(range(min(NFC, k_ * per), min(NFC, (k_ + 1) * per))),
                                   list(range(min(NFC, max(0, k_ - 1) * per), min(NFC, k_ * per))) if k_ > 0 else []))
            done_down = set()
            p_blk(0)
            for gb in range(NB):
                if split:
                    if gb == cfg["wdwait"]:
                        wd_cp.wait()
                elif gb == fwait and fwait > 0:
                    wg_cp.wait(); wu_cp.wait(); wd_cp.wait()
                if gb + 1 < NB:
                    p_blk(gb + 1)
                kvm_blk(gb)
                gus, dns = fsched[gb]
                for c in gus:
                    ffn_gu(c)
                for c in dns:
                    ffn_down(c); done_down.add(c)
                for g in range(gb * gpb, (gb + 1) * gpb):
                    den_piece(0, g)
            for c in range(NFC):
                if c not in done_down:
                    ffn_down(c)
            ffn_fin()

        if cfg.get("bcbar", False):
            bar_cp.wait()
        for i in range(NTILE):
            rows = pl.ds(i * TS, TS)
            for n in range(NOC):
                with scope(f"o{i}"):
                    cols = pl.ds(n * ON, ON)
                    a = _dot(o_v.ld(i * TS, TS), m_v.ld(0, D, n * ON, ON))
                    if i + 1 < NTILE:
                        gpn = G // NOC
                        for g in range(n * gpn, (n + 1) * gpn):
                            den_piece(i + 1, g)
                    out_v[rows, cols] = (res_v[rows, cols] + a).astype(BF)
                    out_cp[(i, n)].start()
        with scope("wait_out"):
            for i in range(NTILE):
                for n in range(NOC):
                    out_cp[(i, n)].wait()

    nsem_total = NPT + NTILE - 1 + NCH + 7 + NTILE * NOC
    pb = lambda r, c: pltpu.VMEM((r // 2, c), U32)
    scratch = [
        pltpu.VMEM((S, D), BF),
        pltpu.VMEM((D, 3 * D), BF),
        pltpu.VMEM((D, D), BF),
        pltpu.VMEM((D,), BF),
        pltpu.VMEM((D, F), BF),
        pltpu.VMEM((D, F), BF),
        pltpu.VMEM((F, D), BF),
        pb(S, D),
        pltpu.VMEM((S, D), F32),
        pb(2 * D, D),
        pb(D, S),
        pb(D, S),
        pb(D, D),
        pb(S, D),
        pb(D, D),
        pltpu.VMEM((D, 128), F32),
        pltpu.VMEM((S, D), BF),
        pltpu.VMEM((D, 128), F32),
        pltpu.VMEM((F, 128), F32),
        pltpu.VMEM((16, D), BF),
        pltpu.SemaphoreType.DMA((nsem_total,)),
    ]

    def fn(A_x, A_wqkv, A_wo, B_x, B_w_r, B_w_gate, B_w_up, B_w_down):
        del B_x
        anyspec = pl.BlockSpec(memory_space=pl.ANY)
        out = pl.pallas_call(
            kernel,
            out_shape=jax.ShapeDtypeStruct((S, D), BF),
            in_specs=[anyspec] * 7,
            out_specs=anyspec,
            scratch_shapes=scratch,
            compiler_params=pltpu.CompilerParams(vmem_limit_bytes=cfg.get("vmem", 110 * 1024 * 1024),
                                                 flags=cfg.get("flags")),
            name=cfg.get("name", "k"),
        )(A_x.reshape(S, D), A_wqkv, A_wo, B_w_r, B_w_gate, B_w_up, B_w_down)
        return out.reshape(1, S, D)

    return jax.jit(fn)


def pallas_parallel_sum__linear_attn_block__moe_arch_mod__prompt_kernel(
    A_x, A_wqkv, A_wo, B_x, B_w_r, B_w_gate, B_w_up, B_w_down,
):
    fn = make_kernel(dict(name='fused', flags={'XLA_TPU_EVENLY_DISTRIBUTE_CRITICAL_NODES': True}, MB=256, ffn='vpu', bcbar=True, fwait=0, FC=256))
    return fn(A_x, A_wqkv, A_wo, B_x, B_w_r, B_w_gate, B_w_up, B_w_down)
```

```python
import numpy as np
import jax
import jax.numpy as jnp
from jax import lax
from jax.experimental import pallas as pl
from jax.experimental.pallas import tpu as pltpu

S, D, DH, F = 2048, 1024, 32, 3584
G = D // 128
TS = 512
NTILE = S // TS
LNP = 128
LNR = 32
SEGS = (1, 2, 4, 5, 4)
NCH = 2 * G
MA = 256
MB = 256
NB = D // MB
WD_WAIT = 2
FC = 256
NFC = F // FC
ON = 256
NOC = D // ON

BF, F32, U32 = jnp.bfloat16, jnp.float32, jnp.uint32
NN = (((1,), (0,)), ((), ()))
NT = (((1,), (1,)), ((), ()))


def _dot(a, b, dn=NN):
    return lax.dot_general(a, b, dn, preferred_element_type=F32)


def _rnd(x):
    return x.astype(BF).astype(F32)


def _phi(t):
    return jnp.where(t > 0, t + 1.0, jnp.exp(t)) + 1e-6


class _Packed:
    def __init__(self, ref):
        self.ref = ref

    def ld(self, r0, nr, c0=0, nc=None):
        nc = self.ref.shape[1] - c0 if nc is None else nc
        if isinstance(r0, int):
            v = self.ref[pl.ds(r0 // 2, nr // 2), pl.ds(c0, nc)]
        else:
            v = self.ref[pl.ds(pl.multiple_of(r0 // 2, 8), nr // 2), pl.ds(c0, nc)]
        return pltpu.bitcast(v, BF)

    def st(self, r0, c0, val):
        nr, nc = val.shape
        self.ref[pl.ds(r0 // 2, nr // 2), pl.ds(c0, nc)] = pltpu.bitcast(val, U32)


def _kernel(x_hbm, wqkv_hbm, wo_hbm, wr_hbm, wg_hbm, wu_hbm, wd_hbm, out_hbm,
            x_v, w_v, wo_v, wr_v, wg_v, wu_v, wd_v, xn_r, res_v, wT_r, pqT_r, pkT_r,
            m_r, o_r, p_r, z_v, out_v, xb_v, hb_v, bar_v, sems):
    xn_v, wT_v, pqT_v, pkT_v, m_v, o_v, p_v = (
        _Packed(r) for r in (xn_r, wT_r, pqT_r, pkT_r, m_r, o_r, p_r))

    nsem = [0]

    def cp(src, dst):
        c = pltpu.make_async_copy(src, dst, sems.at[nsem[0]])
        nsem[0] += 1
        return c

    npt = TS // LNP
    x0_cp = [cp(x_hbm.at[pl.ds(p * LNP, LNP)], x_v.at[pl.ds(p * LNP, LNP)]) for p in range(npt)]
    xt_cp = [None] + [cp(x_hbm.at[pl.ds(i * TS, TS)], x_v.at[pl.ds(i * TS, TS)])
                      for i in range(1, NTILE)]
    w_cp = []
    for c in range(NCH):
        c0 = (c % 2) * D + (c // 2) * 128
        w_cp.append(cp(wqkv_hbm.at[:, pl.ds(c0, 128)], w_v.at[:, pl.ds(c0, 128)]))
    wv_cp = cp(wqkv_hbm.at[:, pl.ds(2 * D, D)], w_v.at[:, pl.ds(2 * D, D)])
    wr_cp = cp(wr_hbm, wr_v)
    wo_cp = cp(wo_hbm, wo_v)
    wg_cp = cp(wg_hbm, wg_v)
    wu_cp = cp(wu_hbm, wu_v)
    wd_cp = cp(wd_hbm, wd_v)
    bar_cp = cp(x_hbm.at[pl.ds(0, 16)], bar_v)
    out_cp = {(i, n): cp(out_v.at[pl.ds(i * TS, TS), pl.ds(n * ON, ON)],
                         out_hbm.at[pl.ds(i * TS, TS), pl.ds(n * ON, ON)])
              for i in range(NTILE) for n in range(NOC)}

    for p in range(npt):
        x0_cp[p].start()
        if p == 0:
            wr_cp.start()
    for c in range(NCH):
        w_cp[c].start()
    for i in range(1, NTILE):
        xt_cp[i].start()
    wv_cp.start()
    bar_cp.start()
    wo_cp.start()
    wg_cp.start()
    wu_cp.start()
    wd_cp.start()

    st = dict(best=None, besti=None)
    grp_iota = lax.broadcasted_iota(jnp.int32, (LNR, 1), 0)

    def ln_xn(r0, n):
        for rr in range(r0, r0 + n, LNR):
            x = x_v[pl.ds(rr, LNR), :].astype(F32)
            m = jnp.mean(x, axis=-1, keepdims=True)
            mb = _rnd(m)
            xc = x - mb
            dm = m - mb
            v = jnp.mean(xc * xc, axis=-1, keepdims=True) - dm * dm
            sd = _rnd(jnp.sqrt(_rnd(_rnd(v) + np.float32(1e-5))))
            xn_v.st(rr, 0, (xc * (1.0 / sd)).astype(BF))

    def ln_post(r0, n):
        wr = st["wr"]
        for rr in range(r0, r0 + n, LNR):
            x = x_v[pl.ds(rr, LNR), :].astype(F32)
            xn = xn_v.ld(rr, LNR).astype(F32)
            res_v[pl.ds(rr, LNR), :] = x + xn
            r = _rnd(jnp.sum(xn * wr, axis=-1, keepdims=True))
            r = jnp.where(r != r, -jnp.inf, r)
            ri = grp_iota + rr
            if st["best"] is None:
                st["best"], st["besti"] = r, ri
            else:
                better = r > st["best"]
                st["best"] = jnp.where(better, r, st["best"])
                st["besti"] = jnp.where(better, ri, st["besti"])

    def spread(fn, r0, n, k, nk):
        ng = n // LNR
        a, b = k * ng // nk, (k + 1) * ng // nk
        if b > a:
            fn(r0 + a * LNR, (b - a) * LNR)

    for p in range(npt):
        x0_cp[p].wait()
        if p == npt - 1:
            wr_cp.wait()
            st["wr"] = wr_v[...].astype(F32).reshape(1, D)
        ln_xn(p * LNP, LNP)

    def proj_t(i, j, r0, nr):
        p = _phi(_dot(wT_v.ld(j * D + r0, nr), xn_v.ld(i * TS, TS), NT))
        if j == 0:
            pqT_v.st(r0, i * TS, p.astype(BF))
            return
        zs = p[:, 0:128]
        for n in range(1, TS // 128):
            zs = zs + p[:, n * 128:(n + 1) * 128]
        if i == 0:
            z_v[pl.ds(r0, nr), :] = zs
        else:
            z_v[pl.ds(r0, nr), :] = z_v[pl.ds(r0, nr), :] + zs
        pkT_v.st(r0, i * TS, p.astype(BF))

    c0 = 0
    for si, sn in enumerate(SEGS):
        for c in range(c0, c0 + sn):
            w_cp[c].wait()
        if si == len(SEGS) - 1:
            xt_cp[1].wait()
        for c in range(c0, c0 + sn):
            g, j = c // 2, c % 2
            wT_v.st(j * D + g * 128, 0, w_v[:, pl.ds(j * D + g * 128, 128)].T)
        for k, c in enumerate(range(c0, c0 + sn)):
            g, j = c // 2, c % 2
            proj_t(0, j, g * 128, 128)
            if si == len(SEGS) - 2:
                spread(ln_post, 0, TS, k, sn)
            if si == len(SEGS) - 1:
                spread(ln_xn, TS, TS, k, sn)
        c0 += sn

    nd = 2 * (D // MA)
    for i in range(1, NTILE):
        if i + 1 < NTILE:
            xt_cp[i + 1].wait()
        if i == NTILE - 1:
            wv_cp.wait()
            wo_cp.wait()
        k = 0
        for rb in range(D // MA):
            for j in range(2):
                proj_t(i, j, rb * MA, MA)
                if i + 1 < NTILE:
                    spread(ln_xn, (i + 1) * TS, TS, k, nd)
                spread(ln_post, i * TS, TS, k, nd)
                k += 1

    head_r = lax.broadcasted_iota(jnp.int32, (128, 128), 0) // DH
    head_c = lax.broadcasted_iota(jnp.int32, (128, 128), 1) // DH
    same_head = head_r == head_c
    zcol = [None] * G
    ffn = {}

    def ffn_prep():
        best, besti = st["best"], st["besti"]
        bm = jnp.max(best, axis=0, keepdims=True)
        bi = jnp.min(jnp.where(best == bm, besti, S), axis=0, keepdims=True)
        idx = jnp.clip(jnp.min(bi), 0, S - 1)
        base = pl.multiple_of((idx // 16) * 16, 16)
        ffn["idx"], ffn["base"], ffn["rmax"] = idx, base, bm
        x16 = xn_v.ld(base, 16).astype(F32)
        sel = (lax.broadcasted_iota(jnp.int32, (16, D), 0) + base) == idx
        xs = jnp.sum(jnp.where(sel, x16, 0.0), axis=0, keepdims=True)
        for b in range(G):
            xb_v[pl.ds(b * 128, 128), :] = jnp.broadcast_to(
                xs[:, b * 128:(b + 1) * 128], (128, 128)).T

    def matvec(w_refs, col_ref, k0, k1, c0_, nc):
        nl = nc // 128
        acc = [[None] * nl for _ in w_refs]
        for kb in range(k0, k1, 8):
            xk = col_ref[pl.ds(kb, 8), :]
            for l2 in range(nl // 2):
                cols = pl.ds(c0_ + l2 * 256, 256)
                for wi, w_ref in enumerate(w_refs):
                    w = w_ref[pl.ds(kb, 8), cols].astype(F32)
                    for t in range(2):
                        pr = w[:, t * 128:(t + 1) * 128] * xk
                        a = acc[wi][2 * l2 + t]
                        acc[wi][2 * l2 + t] = pr if a is None else a + pr
        return acc

    def ffn_gu(c):
        ag, au = matvec([wg_v, wu_v], xb_v, 0, D, c * FC, FC)
        for b in range(FC // 128):
            gt = jnp.sum(ag[b], axis=0, keepdims=True)
            up = jnp.sum(au[b], axis=0, keepdims=True)
            h = gt * jax.nn.sigmoid(gt) * up
            hb_v[pl.ds(c * FC + b * 128, 128), :] = jnp.broadcast_to(h, (128, 128)).T

    def ffn_down(c):
        (ay,) = matvec([wd_v], hb_v, c * FC, (c + 1) * FC, 0, D)
        ay = [pltpu.roll(pltpu.roll(a, 1, 1), 127, 1) for a in ay]
        ffn["ay"] = ay if ffn.get("ay") is None else [a + b for a, b in zip(ffn["ay"], ay)]

    def ffn_fin():
        y = jnp.concatenate([jnp.sum(a, axis=0, keepdims=True) for a in ffn["ay"]], axis=1)
        gate = jax.nn.sigmoid(ffn["rmax"])
        base, idx = ffn["base"], ffn["idx"]
        sel = (lax.broadcasted_iota(jnp.int32, (16, D), 0) + base) == idx
        res_v[pl.ds(base, 16), :] = res_v[pl.ds(base, 16), :] + jnp.where(sel, y * gate, 0.0)

    def normalise(i, g):
        p = pqT_v.ld(g * 128, 128, i * TS, TS).astype(F32)
        zb = jnp.concatenate([zcol[g]] * (TS // 128), axis=1)
        p4 = p.reshape(4, DH, TS)
        den = jnp.sum(p4 * zb.reshape(4, DH, TS), axis=1, keepdims=True) + 1e-6
        o = (p4 * (1.0 / den)).reshape(128, TS).astype(BF)
        o_v.st(i * TS, g * 128, o.T)

    def p_blk(gb):
        p_v.st(gb * MB, 0, _dot(pkT_v.ld(gb * MB, MB), xn_v.ld(0, S)).astype(BF))

    def kvm_blk(gb):
        for g in range(gb * MB // 128, (gb + 1) * MB // 128):
            kv = _dot(p_v.ld(g * 128, 128), w_v[:, pl.ds(2 * D + g * 128, 128)])
            kvm = jnp.where(same_head, kv, 0.0).astype(BF)
            m_v.st(g * 128, 0, _dot(kvm, wo_v[pl.ds(g * 128, 128), :]).astype(BF))

    wg_cp.wait()
    wu_cp.wait()
    ffn_prep()
    for g in range(G):
        zcol[g] = jnp.broadcast_to(
            jnp.sum(z_v[pl.ds(g * 128, 128), :], axis=1, keepdims=True), (128, 128))
    gpb = MB // 128
    p_blk(0)
    for gb in range(NB):
        if gb == WD_WAIT:
            wd_cp.wait()
        if gb + 1 < NB:
            p_blk(gb + 1)
        kvm_blk(gb)
        if gb < WD_WAIT:
            for c in range(gb * NFC // WD_WAIT, (gb + 1) * NFC // WD_WAIT):
                ffn_gu(c)
        else:
            kk, nk = gb - WD_WAIT, NB - WD_WAIT
            for c in range(kk * NFC // nk, (kk + 1) * NFC // nk):
                ffn_down(c)
        for g in range(gb * gpb, (gb + 1) * gpb):
            normalise(0, g)
    ffn_fin()

    bar_cp.wait()
    for i in range(NTILE):
        rows = pl.ds(i * TS, TS)
        for n in range(NOC):
            cols = pl.ds(n * ON, ON)
            a = _dot(o_v.ld(i * TS, TS), m_v.ld(0, D, n * ON, ON))
            if i + 1 < NTILE:
                gpn = G // NOC
                for g in range(n * gpn, (n + 1) * gpn):
                    normalise(i + 1, g)
            out_v[rows, cols] = (res_v[rows, cols] + a).astype(BF)
            out_cp[(i, n)].start()
    for i in range(NTILE):
        for n in range(NOC):
            out_cp[(i, n)].wait()


def _packed(r, c):
    return pltpu.VMEM((r // 2, c), U32)


@jax.jit
def pallas_parallel_sum__linear_attn_block__moe_arch_mod__prompt_kernel(
    A_x, A_wqkv, A_wo, B_x, B_w_r, B_w_gate, B_w_up, B_w_down,
):
    del B_x
    nsem = TS // LNP + (NTILE - 1) + NCH + 7 + NTILE * NOC
    scratch = [
        pltpu.VMEM((S, D), BF),
        pltpu.VMEM((D, 3 * D), BF),
        pltpu.VMEM((D, D), BF),
        pltpu.VMEM((D,), BF),
        pltpu.VMEM((D, F), BF),
        pltpu.VMEM((D, F), BF),
        pltpu.VMEM((F, D), BF),
        _packed(S, D),
        pltpu.VMEM((S, D), F32),
        _packed(2 * D, D),
        _packed(D, S),
        _packed(D, S),
        _packed(D, D),
        _packed(S, D),
        _packed(D, D),
        pltpu.VMEM((D, 128), F32),
        pltpu.VMEM((S, D), BF),
        pltpu.VMEM((D, 128), F32),
        pltpu.VMEM((F, 128), F32),
        pltpu.VMEM((16, D), BF),
        pltpu.SemaphoreType.DMA((nsem,)),
    ]
    any_spec = pl.BlockSpec(memory_space=pl.ANY)
    out = pl.pallas_call(
        _kernel,
        out_shape=jax.ShapeDtypeStruct((S, D), BF),
        in_specs=[any_spec] * 7,
        out_specs=any_spec,
        scratch_shapes=scratch,
        compiler_params=pltpu.CompilerParams(
            vmem_limit_bytes=110 * 1024 * 1024,
            flags={"XLA_TPU_EVENLY_DISTRIBUTE_CRITICAL_NODES": True},
        ),
        name="fused_linattn_mod",
    )(A_x.reshape(S, D), A_wqkv, A_wo, B_w_r, B_w_gate, B_w_up, B_w_down)
    return out.reshape(1, S, D)
```

```python
import numpy as np
import jax
import jax.numpy as jnp
from jax import lax
from jax.experimental import pallas as pl
from jax.experimental.pallas import tpu as pltpu

S, D, DH, F = 2048, 1024, 32, 3584
G = D // 128
TS = 512
NTILE = S // TS
LNP = 128
LNR = 32
SEGS = (1, 2, 4, 5, 4)
X1_POS = 12
X1_SEG = 3
NCH = 2 * G
MA = 256
MB = 256
NB = D // MB
WD_WAIT = 2
FC = 256
GSPLIT = 4
NFC = F // FC
ON = 256
NOC = D // ON
TSPLIT = 2

BF, F32, U32 = jnp.bfloat16, jnp.float32, jnp.uint32
NN = (((1,), (0,)), ((), ()))
NT = (((1,), (1,)), ((), ()))


def _dot(a, b, dn=NN):
    return lax.dot_general(a, b, dn, preferred_element_type=F32)


def _rnd(x):
    return x.astype(BF).astype(F32)


def _phi(t):
    return jnp.where(t > 0, t + 1.0, jnp.exp(t)) + 1e-6


def _xlu_identity(a):
    return pltpu.roll(pltpu.roll(a, 1, 1), 127, 1)


class _Packed:
    def __init__(self, ref):
        self.ref = ref

    def ld(self, r0, nr, c0=0, nc=None):
        nc = self.ref.shape[1] - c0 if nc is None else nc
        if isinstance(r0, int):
            v = self.ref[pl.ds(r0 // 2, nr // 2), pl.ds(c0, nc)]
        else:
            v = self.ref[pl.ds(pl.multiple_of(r0 // 2, 8), nr // 2), pl.ds(c0, nc)]
        return pltpu.bitcast(v, BF)

    def st(self, r0, c0, val):
        nr, nc = val.shape
        self.ref[pl.ds(r0 // 2, nr // 2), pl.ds(c0, nc)] = pltpu.bitcast(val, U32)


def _kernel(x_hbm, wqkv_hbm, wo_hbm, wr_hbm, wg_hbm, wu_hbm, wd_hbm, out_hbm,
            x_v, w_v, wo_v, wr_v, wg_v, wu_v, wd_v, xn_r, res_v, wT_r, pqT_r, pkT_r,
            m_r, o_r, p_r, z_v, out_v, xb_v, hb_v, bar_v, sems):
    xn_v, wT_v, pqT_v, pkT_v, m_v, o_v, p_v = (
        _Packed(r) for r in (xn_r, wT_r, pqT_r, pkT_r, m_r, o_r, p_r))

    nsem = [0]

    def cp(src, dst):
        c = pltpu.make_async_copy(src, dst, sems.at[nsem[0]])
        nsem[0] += 1
        return c

    npt = TS // LNP
    x0_cp = [cp(x_hbm.at[pl.ds(p * LNP, LNP)], x_v.at[pl.ds(p * LNP, LNP)]) for p in range(npt)]
    xt_cp = [None] + [cp(x_hbm.at[pl.ds(i * TS, TS)], x_v.at[pl.ds(i * TS, TS)])
                      for i in range(1, NTILE)]
    w_cp = []
    for c in range(NCH):
        c0 = (c % 2) * D + (c // 2) * 128
        w_cp.append(cp(wqkv_hbm.at[:, pl.ds(c0, 128)], w_v.at[:, pl.ds(c0, 128)]))
    wv_cp = cp(wqkv_hbm.at[:, pl.ds(2 * D, D)], w_v.at[:, pl.ds(2 * D, D)])
    wr_cp = cp(wr_hbm, wr_v)
    wo_cp = cp(wo_hbm, wo_v)
    wg_cp = cp(wg_hbm, wg_v)
    wu_cp = cp(wu_hbm, wu_v)
    wd_cp = cp(wd_hbm, wd_v)
    bar_cp = cp(x_hbm.at[pl.ds(0, 16)], bar_v)
    out_cp = {(i, n): cp(out_v.at[pl.ds(i * TS, TS), pl.ds(n * ON, ON)],
                         out_hbm.at[pl.ds(i * TS, TS), pl.ds(n * ON, ON)])
              for i in range(NTILE) for n in range(NOC) if (i, n) != (NTILE - 1, NOC - 1)}
    rs = TS // TSPLIT
    tail_cp = [cp(out_v.at[pl.ds(S - TS + t * rs, rs), pl.ds(D - ON, ON)],
                  out_hbm.at[pl.ds(S - TS + t * rs, rs), pl.ds(D - ON, ON)])
               for t in range(TSPLIT)]

    for p in range(npt):
        x0_cp[p].start()
        if p == 0:
            wr_cp.start()
    for c in range(NCH):
        if c == X1_POS:
            xt_cp[1].start()
        w_cp[c].start()
    for i in range(2, NTILE):
        xt_cp[i].start()
    wv_cp.start()
    bar_cp.start()
    wo_cp.start()
    wg_cp.start()
    wu_cp.start()
    wd_cp.start()

    st = dict(best=None, besti=None)
    grp_iota = lax.broadcasted_iota(jnp.int32, (LNR, 1), 0)

    def ln_xn(r0, n):
        for rr in range(r0, r0 + n, LNR):
            x = x_v[pl.ds(rr, LNR), :].astype(F32)
            m = jnp.mean(x, axis=-1, keepdims=True)
            mb = _rnd(m)
            xc = x - mb
            dm = m - mb
            v = jnp.mean(xc * xc, axis=-1, keepdims=True) - dm * dm
            sd = _rnd(jnp.sqrt(_rnd(_rnd(v) + np.float32(1e-5))))
            xn_v.st(rr, 0, (xc * (1.0 / sd)).astype(BF))

    def ln_post(r0, n):
        wr = st["wr"]
        for rr in range(r0, r0 + n, LNR):
            x = x_v[pl.ds(rr, LNR), :].astype(F32)
            xn = xn_v.ld(rr, LNR).astype(F32)
            res_v[pl.ds(rr, LNR), :] = x + xn
            r = _rnd(jnp.sum(xn * wr, axis=-1, keepdims=True))
            r = jnp.where(r != r, -jnp.inf, r)
            ri = grp_iota + rr
            if st["best"] is None:
                st["best"], st["besti"] = r, ri
            else:
                better = r > st["best"]
                st["best"] = jnp.where(better, r, st["best"])
                st["besti"] = jnp.where(better, ri, st["besti"])

    def spread(fn, r0, n, k, nk):
        ng = n // LNR
        a, b = k * ng // nk, (k + 1) * ng // nk
        if b > a:
            fn(r0 + a * LNR, (b - a) * LNR)

    for p in range(npt):
        x0_cp[p].wait()
        if p == npt - 1:
            wr_cp.wait()
            st["wr"] = wr_v[...].astype(F32).reshape(1, D)
        ln_xn(p * LNP, LNP)

    def proj_t(i, j, r0, nr):
        p = _phi(_dot(wT_v.ld(j * D + r0, nr), xn_v.ld(i * TS, TS), NT))
        if j == 0:
            pqT_v.st(r0, i * TS, p.astype(BF))
            return
        zs = p[:, 0:128]
        for n in range(1, TS // 128):
            zs = zs + p[:, n * 128:(n + 1) * 128]
        if i == 0:
            z_v[pl.ds(r0, nr), :] = zs
        else:
            z_v[pl.ds(r0, nr), :] = z_v[pl.ds(r0, nr), :] + zs
        pkT_v.st(r0, i * TS, p.astype(BF))

    c0 = 0
    for si, sn in enumerate(SEGS):
        for c in range(c0, c0 + sn):
            w_cp[c].wait()
        if si == X1_SEG:
            xt_cp[1].wait()
        for c in range(c0, c0 + sn):
            g, j = c // 2, c % 2
            wT_v.st(j * D + g * 128, 0, w_v[:, pl.ds(j * D + g * 128, 128)].T)
        for k, c in enumerate(range(c0, c0 + sn)):
            g, j = c // 2, c % 2
            proj_t(0, j, g * 128, 128)
            if si >= X1_SEG:
                spread(ln_xn, TS, TS, sum(SEGS[X1_SEG:si]) + k, sum(SEGS[X1_SEG:]))
        c0 += sn

    nd = 2 * (D // MA)
    for i in range(1, NTILE):
        if i + 1 < NTILE:
            xt_cp[i + 1].wait()
        if i == NTILE - 1:
            wv_cp.wait()
            wo_cp.wait()
        k = 0
        for rb in range(D // MA):
            for j in range(2):
                proj_t(i, j, rb * MA, MA)
                if i + 1 < NTILE:
                    spread(ln_xn, (i + 1) * TS, TS, k, nd)
                spread(ln_post, i * TS, TS, k, nd)
                if i == NTILE - 1:
                    spread(ln_post, 0, TS, k, nd)
                k += 1

    head_r = lax.broadcasted_iota(jnp.int32, (128, 128), 0) // DH
    head_c = lax.broadcasted_iota(jnp.int32, (128, 128), 1) // DH
    same_head = head_r == head_c
    zcol = [None] * G
    ffn = {}

    def ffn_prep():
        best, besti = st["best"], st["besti"]
        bm = jnp.max(best, axis=0, keepdims=True)
        bi = jnp.min(jnp.where(best == bm, besti, S), axis=0, keepdims=True)
        idx = jnp.clip(jnp.min(bi), 0, S - 1)
        base = pl.multiple_of((idx // 16) * 16, 16)
        ffn["idx"], ffn["base"], ffn["rmax"] = idx, base, bm
        x16 = xn_v.ld(base, 16).astype(F32)
        sel = (lax.broadcasted_iota(jnp.int32, (16, D), 0) + base) == idx
        xs = jnp.sum(jnp.where(sel, x16, 0.0), axis=0, keepdims=True)
        for b in range(G):
            xb_v[pl.ds(b * 128, 128), :] = jnp.broadcast_to(
                xs[:, b * 128:(b + 1) * 128], (128, 128)).T

    def matvec(w_refs, col_ref, k0, k1, c0_, nc):
        nl = nc // 128
        acc = [[None] * nl for _ in w_refs]
        for kb in range(k0, k1, 8):
            xk = col_ref[pl.ds(kb, 8), :]
            for l2 in range(nl // 2):
                cols = pl.ds(c0_ + l2 * 256, 256)
                for wi, w_ref in enumerate(w_refs):
                    w = w_ref[pl.ds(kb, 8), cols].astype(F32)
                    for t in range(2):
                        pr = w[:, t * 128:(t + 1) * 128] * xk
                        a = acc[wi][2 * l2 + t]
                        acc[wi][2 * l2 + t] = pr if a is None else a + pr
        return acc

    def ffn_gu(c):
        ag = au = None
        for q in range(GSPLIT):
            a1, u1 = matvec([wg_v, wu_v], xb_v, q * D // GSPLIT, (q + 1) * D // GSPLIT, c * FC, FC)
            if q + 1 < GSPLIT:
                a1 = [_xlu_identity(a) for a in a1]
            ag = a1 if ag is None else [a + b for a, b in zip(ag, a1)]
            au = u1 if au is None else [a + b for a, b in zip(au, u1)]
        for b in range(FC // 128):
            gt = jnp.sum(ag[b], axis=0, keepdims=True)
            up = jnp.sum(au[b], axis=0, keepdims=True)
            h = gt * jax.nn.sigmoid(gt) * up
            hb_v[pl.ds(c * FC + b * 128, 128), :] = jnp.broadcast_to(h, (128, 128)).T

    def ffn_down(c):
        (ay,) = matvec([wd_v], hb_v, c * FC, (c + 1) * FC, 0, D)
        ay = [_xlu_identity(a) for a in ay]
        ffn["ay"] = ay if ffn.get("ay") is None else [a + b for a, b in zip(ffn["ay"], ay)]

    def ffn_fin():
        y = jnp.concatenate([jnp.sum(a, axis=0, keepdims=True) for a in ffn["ay"]], axis=1)
        gate = jax.nn.sigmoid(ffn["rmax"])
        base, idx = ffn["base"], ffn["idx"]
        sel = (lax.broadcasted_iota(jnp.int32, (16, D), 0) + base) == idx
        res_v[pl.ds(base, 16), :] = res_v[pl.ds(base, 16), :] + jnp.where(sel, y * gate, 0.0)

    def normalise(i, g):
        p = pqT_v.ld(g * 128, 128, i * TS, TS).astype(F32)
        zb = jnp.concatenate([zcol[g]] * (TS // 128), axis=1)
        p4 = p.reshape(4, DH, TS)
        den = jnp.sum(p4 * zb.reshape(4, DH, TS), axis=1, keepdims=True) + 1e-6
        o = (p4 * (1.0 / den)).reshape(128, TS).astype(BF)
        o_v.st(i * TS, g * 128, o.T)

    def p_blk(gb):
        p_v.st(gb * MB, 0, _dot(pkT_v.ld(gb * MB, MB), xn_v.ld(0, S)).astype(BF))

    def kvm_blk(gb):
        for g in range(gb * MB // 128, (gb + 1) * MB // 128):
            kv = _dot(p_v.ld(g * 128, 128), w_v[:, pl.ds(2 * D + g * 128, 128)])
            kvm = jnp.where(same_head, kv, 0.0).astype(BF)
            m_v.st(g * 128, 0, _dot(kvm, wo_v[pl.ds(g * 128, 128), :]).astype(BF))

    wg_cp.wait()
    wu_cp.wait()
    ffn_prep()
    for g in range(G):
        zcol[g] = jnp.broadcast_to(
            jnp.sum(z_v[pl.ds(g * 128, 128), :], axis=1, keepdims=True), (128, 128))
    gpb = MB // 128
    p_blk(0)
    for gb in range(NB):
        if gb == WD_WAIT:
            wd_cp.wait()
        if gb + 1 < NB:
            p_blk(gb + 1)
        kvm_blk(gb)
        if gb < WD_WAIT:
            for c in range(gb * NFC // WD_WAIT, (gb + 1) * NFC // WD_WAIT):
                ffn_gu(c)
        else:
            kk, nk = gb - WD_WAIT, NB - WD_WAIT
            for c in range(kk * NFC // nk, (kk + 1) * NFC // nk):
                ffn_down(c)
        for g in range(gb * gpb, (gb + 1) * gpb):
            normalise(0, g)
    ffn_fin()

    bar_cp.wait()
    for i in range(NTILE):
        rows = pl.ds(i * TS, TS)
        for n in range(NOC):
            cols = pl.ds(n * ON, ON)
            if (i, n) == (NTILE - 1, NOC - 1):
                for t in range(TSPLIT):
                    r0 = i * TS + t * rs
                    a = _dot(o_v.ld(r0, rs), m_v.ld(0, D, n * ON, ON))
                    out_v[pl.ds(r0, rs), cols] = (res_v[pl.ds(r0, rs), cols] + a).astype(BF)
                    tail_cp[t].start()
                continue
            a = _dot(o_v.ld(i * TS, TS), m_v.ld(0, D, n * ON, ON))
            if i + 1 < NTILE:
                gpn = G // NOC
                for g in range(n * gpn, (n + 1) * gpn):
                    normalise(i + 1, g)
            out_v[rows, cols] = (res_v[rows, cols] + a).astype(BF)
            out_cp[(i, n)].start()
    for c in out_cp.values():
        c.wait()
    for c in tail_cp:
        c.wait()


def _packed(r, c):
    return pltpu.VMEM((r // 2, c), U32)


@jax.jit
def pallas_parallel_sum__linear_attn_block__moe_arch_mod__prompt_kernel(
    A_x, A_wqkv, A_wo, B_x, B_w_r, B_w_gate, B_w_up, B_w_down,
):
    del B_x
    nsem = TS // LNP + (NTILE - 1) + NCH + 7 + NTILE * NOC - 1 + TSPLIT
    scratch = [
        pltpu.VMEM((S, D), BF),
        pltpu.VMEM((D, 3 * D), BF),
        pltpu.VMEM((D, D), BF),
        pltpu.VMEM((D,), BF),
        pltpu.VMEM((D, F), BF),
        pltpu.VMEM((D, F), BF),
        pltpu.VMEM((F, D), BF),
        _packed(S, D),
        pltpu.VMEM((S, D), F32),
        _packed(2 * D, D),
        _packed(D, S),
        _packed(D, S),
        _packed(D, D),
        _packed(S, D),
        _packed(D, D),
        pltpu.VMEM((D, 128), F32),
        pltpu.VMEM((S, D), BF),
        pltpu.VMEM((D, 128), F32),
        pltpu.VMEM((F, 128), F32),
        pltpu.VMEM((16, D), BF),
        pltpu.SemaphoreType.DMA((nsem,)),
    ]
    any_spec = pl.BlockSpec(memory_space=pl.ANY)
    out = pl.pallas_call(
        _kernel,
        out_shape=jax.ShapeDtypeStruct((S, D), BF),
        in_specs=[any_spec] * 7,
        out_specs=any_spec,
        scratch_shapes=scratch,
        compiler_params=pltpu.CompilerParams(
            vmem_limit_bytes=110 * 1024 * 1024,
            flags={"XLA_TPU_EVENLY_DISTRIBUTE_CRITICAL_NODES": True},
        ),
        name="fused_linattn_mod",
    )(A_x.reshape(S, D), A_wqkv, A_wo, B_w_r, B_w_gate, B_w_up, B_w_down)
    return out.reshape(1, S, D)
```

```python
import numpy as np
import jax
import jax.numpy as jnp
from jax import lax
from jax.experimental import pallas as pl
from jax.experimental.pallas import tpu as pltpu

S, D, DH, F = 2048, 1024, 32, 3584
G = D // 128
TS = 512
NTILE = S // TS
LNP = 128
LNR = 64
SEGS = (2, 2, 4, 4, 4)
Q0_POS = 2
X1_POS = 12
X1_SEG = 3
NCH = 2 * G
MA = 256
MB = 256
NB = D // MB
WD_WAIT = 2
FC = 256
GSPLIT = 4
NFC = F // FC
ON = 256
NOC = D // ON
TSPLIT = 2

BF, F32, U32 = jnp.bfloat16, jnp.float32, jnp.uint32
NN = (((1,), (0,)), ((), ()))
NT = (((1,), (1,)), ((), ()))


def _dot(a, b, dn=NN):
    return lax.dot_general(a, b, dn, preferred_element_type=F32)


def _rnd(x):
    return x.astype(BF).astype(F32)


def _phi(t):
    return jnp.where(t > 0, t + 1.0, jnp.exp(t)) + 1e-6


def _xlu_identity(a):
    return pltpu.roll(pltpu.roll(a, 1, 1), 127, 1)


class _Packed:
    def __init__(self, ref):
        self.ref = ref

    def ld(self, r0, nr, c0=0, nc=None):
        nc = self.ref.shape[1] - c0 if nc is None else nc
        if isinstance(r0, int):
            v = self.ref[pl.ds(r0 // 2, nr // 2), pl.ds(c0, nc)]
        else:
            v = self.ref[pl.ds(pl.multiple_of(r0 // 2, 8), nr // 2), pl.ds(c0, nc)]
        return pltpu.bitcast(v, BF)

    def st(self, r0, c0, val):
        nr, nc = val.shape
        self.ref[pl.ds(r0 // 2, nr // 2), pl.ds(c0, nc)] = pltpu.bitcast(val, U32)


def _kernel(x_hbm, wqkv_hbm, wo_hbm, wr_hbm, wg_hbm, wu_hbm, wd_hbm, out_hbm,
            x_v, w_v, wo_v, wr_v, wg_v, wu_v, wd_v, xn_r, res_v, wT_r, pqT_r, pkT_r,
            m_r, o_r, p_r, z_v, out_v, xb_v, hb_v, bar_v, sems):
    xn_v, wT_v, pqT_v, pkT_v, m_v, o_v, p_v = (
        _Packed(r) for r in (xn_r, wT_r, pqT_r, pkT_r, m_r, o_r, p_r))

    nsem = [0]

    def cp(src, dst):
        c = pltpu.make_async_copy(src, dst, sems.at[nsem[0]])
        nsem[0] += 1
        return c

    npt = TS // LNP
    x0_cp = [cp(x_hbm.at[pl.ds(p * LNP, LNP)], x_v.at[pl.ds(p * LNP, LNP)]) for p in range(npt)]
    xt_cp = [None] + [cp(x_hbm.at[pl.ds(i * TS, TS)], x_v.at[pl.ds(i * TS, TS)])
                      for i in range(1, NTILE)]
    w_cp = []
    for c in range(NCH):
        c0 = (c % 2) * D + (c // 2) * 128
        w_cp.append(cp(wqkv_hbm.at[:, pl.ds(c0, 128)], w_v.at[:, pl.ds(c0, 128)]))
    wv_cp = cp(wqkv_hbm.at[:, pl.ds(2 * D, D)], w_v.at[:, pl.ds(2 * D, D)])
    wr_cp = cp(wr_hbm, wr_v)
    wo_cp = cp(wo_hbm, wo_v)
    wg_cp = cp(wg_hbm, wg_v)
    wu_cp = cp(wu_hbm, wu_v)
    wd_cp = cp(wd_hbm, wd_v)
    bar_cp = cp(x_hbm.at[pl.ds(0, 16)], bar_v)
    out_cp = {(i, n): cp(out_v.at[pl.ds(i * TS, TS), pl.ds(n * ON, ON)],
                         out_hbm.at[pl.ds(i * TS, TS), pl.ds(n * ON, ON)])
              for i in range(NTILE) for n in range(NOC) if (i, n) != (NTILE - 1, NOC - 1)}
    rs = TS // TSPLIT
    tail_cp = [cp(out_v.at[pl.ds(S - TS + t * rs, rs), pl.ds(D - ON, ON)],
                  out_hbm.at[pl.ds(S - TS + t * rs, rs), pl.ds(D - ON, ON)])
               for t in range(TSPLIT)]

    for p in range(npt):
        x0_cp[p].start()
        if p == 0:
            wr_cp.start()
        if p == Q0_POS - 1:
            w_cp[0].start()
    for c in range(1, NCH):
        if c == X1_POS:
            xt_cp[1].start()
        w_cp[c].start()
    for i in range(2, NTILE):
        xt_cp[i].start()
    wv_cp.start()
    bar_cp.start()
    wo_cp.start()
    wg_cp.start()
    wu_cp.start()
    wd_cp.start()

    st = dict(best=None, besti=None)
    grp_iota = lax.broadcasted_iota(jnp.int32, (LNR, 1), 0)

    def ln_xn(r0, n):
        for rr in range(r0, r0 + n, LNR):
            x = x_v[pl.ds(rr, LNR), :].astype(F32)
            m = jnp.mean(x, axis=-1, keepdims=True)
            mb = _rnd(m)
            xc = x - mb
            dm = m - mb
            v = jnp.mean(xc * xc, axis=-1, keepdims=True) - dm * dm
            sd = _rnd(jnp.sqrt(_rnd(_rnd(v) + np.float32(1e-5))))
            xn_v.st(rr, 0, (xc * (1.0 / sd)).astype(BF))

    def ln_post(r0, n):
        wr = st["wr"]
        for rr in range(r0, r0 + n, LNR):
            x = x_v[pl.ds(rr, LNR), :].astype(F32)
            xn = xn_v.ld(rr, LNR).astype(F32)
            res_v[pl.ds(rr, LNR), :] = x + xn
            r = _rnd(jnp.sum(xn * wr, axis=-1, keepdims=True))
            r = jnp.where(r != r, -jnp.inf, r)
            ri = grp_iota + rr
            if st["best"] is None:
                st["best"], st["besti"] = r, ri
            else:
                better = (r > st["best"]) | ((r == st["best"]) & (ri < st["besti"]))
                st["best"] = jnp.where(better, r, st["best"])
                st["besti"] = jnp.where(better, ri, st["besti"])

    def spread(fn, r0, n, k, nk):
        ng = n // LNR
        a, b = k * ng // nk, (k + 1) * ng // nk
        if b > a:
            fn(r0 + a * LNR, (b - a) * LNR)

    def q0_piece(p):
        t = _dot(wT_v.ld(0, 128), xn_v.ld(p * LNP, LNP), NT)
        pqT_v.st(0, p * LNP, _phi(t).astype(BF))

    for p in range(npt):
        x0_cp[p].wait()
        if p == npt - 1:
            wr_cp.wait()
            st["wr"] = wr_v[...].astype(F32).reshape(1, D)
        if p == Q0_POS:
            w_cp[0].wait()
            wT_v.st(0, 0, w_v[:, pl.ds(0, 128)].T)
        ln_xn(p * LNP, LNP)
        if p == Q0_POS:
            for pp in range(p):
                q0_piece(pp)
        elif p > Q0_POS:
            q0_piece(p - 1)

    def proj_t(i, j, r0, nr):
        p = _phi(_dot(wT_v.ld(j * D + r0, nr), xn_v.ld(i * TS, TS), NT))
        if j == 0:
            pqT_v.st(r0, i * TS, p.astype(BF))
            return
        zs = p[:, 0:128]
        for n in range(1, TS // 128):
            zs = zs + p[:, n * 128:(n + 1) * 128]
        if i == 0:
            z_v[pl.ds(r0, nr), :] = zs
        else:
            z_v[pl.ds(r0, nr), :] = z_v[pl.ds(r0, nr), :] + zs
        pkT_v.st(r0, i * TS, p.astype(BF))

    c0 = 0
    for si, sn in enumerate(SEGS):
        for c in range(max(c0, 1), c0 + sn):
            w_cp[c].wait()
        if si == X1_SEG:
            xt_cp[1].wait()
        for c in range(max(c0, 1), c0 + sn):
            g, j = c // 2, c % 2
            wT_v.st(j * D + g * 128, 0, w_v[:, pl.ds(j * D + g * 128, 128)].T)
        for k, c in enumerate(range(c0, c0 + sn)):
            g, j = c // 2, c % 2
            if c == 0:
                q0_piece(npt - 1)
            else:
                proj_t(0, j, g * 128, 128)
            if si >= X1_SEG:
                spread(ln_xn, TS, TS, sum(SEGS[X1_SEG:si]) + k, sum(SEGS[X1_SEG:]))
        c0 += sn

    nd = 2 * (D // MA)
    for i in range(1, NTILE):
        if i + 1 < NTILE:
            xt_cp[i + 1].wait()
        if i == NTILE - 1:
            wv_cp.wait()
            wo_cp.wait()
        k = 0
        for rb in range(D // MA):
            for j in range(2):
                proj_t(i, j, rb * MA, MA)
                if i + 1 < NTILE:
                    spread(ln_xn, (i + 1) * TS, TS, k, nd)
                spread(ln_post, i * TS, TS, k, nd)
                if i == NTILE - 1:
                    spread(ln_post, 0, TS, k, nd)
                k += 1

    head_r = lax.broadcasted_iota(jnp.int32, (128, 128), 0) // DH
    head_c = lax.broadcasted_iota(jnp.int32, (128, 128), 1) // DH
    same_head = head_r == head_c
    zcol = [None] * G
    ffn = {}

    def ffn_prep():
        best, besti = st["best"], st["besti"]
        bm = jnp.max(best, axis=0, keepdims=True)
        bi = jnp.min(jnp.where(best == bm, besti, S), axis=0, keepdims=True)
        idx = jnp.clip(jnp.min(bi), 0, S - 1)
        base = pl.multiple_of((idx // 16) * 16, 16)
        ffn["idx"], ffn["base"], ffn["rmax"] = idx, base, bm
        x16 = xn_v.ld(base, 16).astype(F32)
        sel = (lax.broadcasted_iota(jnp.int32, (16, D), 0) + base) == idx
        xs = jnp.sum(jnp.where(sel, x16, 0.0), axis=0, keepdims=True)
        for b in range(G):
            xb_v[pl.ds(b * 128, 128), :] = jnp.broadcast_to(
                xs[:, b * 128:(b + 1) * 128], (128, 128)).T

    def matvec(w_refs, col_ref, k0, k1, c0_, nc):
        nl = nc // 128
        acc = [[None] * nl for _ in w_refs]
        for kb in range(k0, k1, 8):
            xk = col_ref[pl.ds(kb, 8), :]
            for l2 in range(nl // 2):
                cols = pl.ds(c0_ + l2 * 256, 256)
                for wi, w_ref in enumerate(w_refs):
                    w = w_ref[pl.ds(kb, 8), cols].astype(F32)
                    for t in range(2):
                        pr = w[:, t * 128:(t + 1) * 128] * xk
                        a = acc[wi][2 * l2 + t]
                        acc[wi][2 * l2 + t] = pr if a is None else a + pr
        return acc

    def ffn_gu(c):
        ag = au = None
        for q in range(GSPLIT):
            a1, u1 = matvec([wg_v, wu_v], xb_v, q * D // GSPLIT, (q + 1) * D // GSPLIT, c * FC, FC)
            if q + 1 < GSPLIT:
                a1 = [_xlu_identity(a) for a in a1]
            ag = a1 if ag is None else [a + b for a, b in zip(ag, a1)]
            au = u1 if au is None else [a + b for a, b in zip(au, u1)]
        for b in range(FC // 128):
            gt = jnp.sum(ag[b], axis=0, keepdims=True)
            up = jnp.sum(au[b], axis=0, keepdims=True)
            h = gt * jax.nn.sigmoid(gt) * up
            hb_v[pl.ds(c * FC + b * 128, 128), :] = jnp.broadcast_to(h, (128, 128)).T

    def ffn_down(c):
        (ay,) = matvec([wd_v], hb_v, c * FC, (c + 1) * FC, 0, D)
        ay = [_xlu_identity(a) for a in ay]
        ffn["ay"] = ay if ffn.get("ay") is None else [a + b for a, b in zip(ffn["ay"], ay)]

    def ffn_fin():
        y = jnp.concatenate([jnp.sum(a, axis=0, keepdims=True) for a in ffn["ay"]], axis=1)
        gate = jax.nn.sigmoid(ffn["rmax"])
        base, idx = ffn["base"], ffn["idx"]
        sel = (lax.broadcasted_iota(jnp.int32, (16, D), 0) + base) == idx
        res_v[pl.ds(base, 16), :] = res_v[pl.ds(base, 16), :] + jnp.where(sel, y * gate, 0.0)

    def normalise(i, g):
        p = pqT_v.ld(g * 128, 128, i * TS, TS).astype(F32)
        zb = jnp.concatenate([zcol[g]] * (TS // 128), axis=1)
        p4 = p.reshape(4, DH, TS)
        den = jnp.sum(p4 * zb.reshape(4, DH, TS), axis=1, keepdims=True) + 1e-6
        o = (p4 * (1.0 / den)).reshape(128, TS).astype(BF)
        o_v.st(i * TS, g * 128, o.T)

    def p_blk(gb):
        p_v.st(gb * MB, 0, _dot(pkT_v.ld(gb * MB, MB), xn_v.ld(0, S)).astype(BF))

    def kvm_blk(gb):
        for g in range(gb * MB // 128, (gb + 1) * MB // 128):
            kv = _dot(p_v.ld(g * 128, 128), w_v[:, pl.ds(2 * D + g * 128, 128)])
            kvm = jnp.where(same_head, kv, 0.0).astype(BF)
            m_v.st(g * 128, 0, _dot(kvm, wo_v[pl.ds(g * 128, 128), :]).astype(BF))

    wg_cp.wait()
    wu_cp.wait()
    ffn_prep()
    for g in range(G):
        zcol[g] = jnp.broadcast_to(
            jnp.sum(z_v[pl.ds(g * 128, 128), :], axis=1, keepdims=True), (128, 128))
    gpb = MB // 128
    p_blk(0)
    for gb in range(NB):
        if gb == WD_WAIT:
            wd_cp.wait()
        if gb + 1 < NB:
            p_blk(gb + 1)
        kvm_blk(gb)
        if gb < WD_WAIT:
            for c in range(gb * NFC // WD_WAIT, (gb + 1) * NFC // WD_WAIT):
                ffn_gu(c)
        else:
            kk, nk = gb - WD_WAIT, NB - WD_WAIT
            for c in range(kk * NFC // nk, (kk + 1) * NFC // nk):
                ffn_down(c)
        for g in range(gb * gpb, (gb + 1) * gpb):
            normalise(0, g)
    ffn_fin()

    bar_cp.wait()
    for i in range(NTILE):
        rows = pl.ds(i * TS, TS)
        for n in range(NOC):
            cols = pl.ds(n * ON, ON)
            if (i, n) == (NTILE - 1, NOC - 1):
                for t in range(TSPLIT):
                    r0 = i * TS + t * rs
                    a = _dot(o_v.ld(r0, rs), m_v.ld(0, D, n * ON, ON))
                    out_v[pl.ds(r0, rs), cols] = (res_v[pl.ds(r0, rs), cols] + a).astype(BF)
                    tail_cp[t].start()
                continue
            a = _dot(o_v.ld(i * TS, TS), m_v.ld(0, D, n * ON, ON))
            if i + 1 < NTILE:
                gpn = G // NOC
                for g in range(n * gpn, (n + 1) * gpn):
                    normalise(i + 1, g)
            out_v[rows, cols] = (res_v[rows, cols] + a).astype(BF)
            out_cp[(i, n)].start()
    for c in out_cp.values():
        c.wait()
    for c in tail_cp:
        c.wait()


def _packed(r, c):
    return pltpu.VMEM((r // 2, c), U32)


@jax.jit
def pallas_parallel_sum__linear_attn_block__moe_arch_mod__prompt_kernel(
    A_x, A_wqkv, A_wo, B_x, B_w_r, B_w_gate, B_w_up, B_w_down,
):
    del B_x
    nsem = TS // LNP + (NTILE - 1) + NCH + 7 + NTILE * NOC - 1 + TSPLIT
    scratch = [
        pltpu.VMEM((S, D), BF),
        pltpu.VMEM((D, 3 * D), BF),
        pltpu.VMEM((D, D), BF),
        pltpu.VMEM((D,), BF),
        pltpu.VMEM((D, F), BF),
        pltpu.VMEM((D, F), BF),
        pltpu.VMEM((F, D), BF),
        _packed(S, D),
        pltpu.VMEM((S, D), F32),
        _packed(2 * D, D),
        _packed(D, S),
        _packed(D, S),
        _packed(D, D),
        _packed(S, D),
        _packed(D, D),
        pltpu.VMEM((D, 128), F32),
        pltpu.VMEM((S, D), BF),
        pltpu.VMEM((D, 128), F32),
        pltpu.VMEM((F, 128), F32),
        pltpu.VMEM((16, D), BF),
        pltpu.SemaphoreType.DMA((nsem,)),
    ]
    any_spec = pl.BlockSpec(memory_space=pl.ANY)
    out = pl.pallas_call(
        _kernel,
        out_shape=jax.ShapeDtypeStruct((S, D), BF),
        in_specs=[any_spec] * 7,
        out_specs=any_spec,
        scratch_shapes=scratch,
        compiler_params=pltpu.CompilerParams(
            vmem_limit_bytes=110 * 1024 * 1024,
            flags={"XLA_TPU_EVENLY_DISTRIBUTE_CRITICAL_NODES": True},
        ),
        name="fused_linattn_mod",
    )(A_x.reshape(S, D), A_wqkv, A_wo, B_w_r, B_w_gate, B_w_up, B_w_down)
    return out.reshape(1, S, D)
```
